```python
import os as _os
_os.environ.setdefault("JAX_PLATFORMS", "cpu")
import jax
import jax.numpy as jnp

def _softmax(x, axis=-1):
    return jax.nn.softmax(x, axis=axis)
def _gelu(x):
    return jax.nn.gelu(x, approximate=True)
def _silu(x):
    return jax.nn.silu(x)
def _sigmoid(x):
    return jax.nn.sigmoid(x)
def _layernorm(x, axis=-1, eps=1e-5):
    m = jnp.mean(x, axis=axis, keepdims=True)
    v = jnp.var(x, axis=axis, keepdims=True)
    return (x - m) / jnp.sqrt(v + eps)
def _scatter_add(tgt, idx, src, axis=0):
    return tgt.at[idx].add(src)
def _segment_sum(src, seg, n):
    return jax.ops.segment_sum(src, seg, n)
class _Rng:
    def __init__(self, key):
        self._k = key
    def _next(self):
        self._k, sub = jax.random.split(self._k)
        return sub
    def normal(self, shape):
        return jax.random.normal(self._next(), shape, dtype=jnp.bfloat16)
    def randint(self, lo, hi, shape):
        return jax.random.randint(self._next(), shape, lo, hi, dtype=jnp.int32)
    def uniform(self, shape, lo=0.0, hi=1.0):
        return jax.random.uniform(self._next(), shape, jnp.bfloat16, lo, hi)
    def permutation(self, n):
        return jax.random.permutation(self._next(), n)


kernel_name = 'gated_mix__sliding_local_dilated__linear_attn_block__prompt'

def setup_inputs():
    _rng = _Rng(jax.random.key(int.from_bytes(__import__("os").urandom(4), "little")))
    _w = (lambda a: (lambda t: t.astype(jnp.bfloat16) if jnp.issubdtype(t.dtype, jnp.floating) else t)(jnp.asarray(a)))
    def _A_setup():
        B, S, D = 1, 2048, 448
        return {
            "x": _w((lambda *s: _rng.normal(s) * 0.05)(B, S, D)),
            "wqkv": _w((lambda *s: _rng.normal(s) * 0.8)(D, 3 * D)),
            "wo": _w((lambda *s: _rng.normal(s) * 0.05)(D, D)),
        }
    _A_in = _A_setup()

    def _B_setup():
        B, S, D = 1, 2048, 448
        return {
            "x": _w((lambda *s: _rng.normal(s) * 0.05)(B, S, D)),
            "wqkv": _w((lambda *s: _rng.normal(s) * 1.6)(D, 3 * D)),
            "wo": _w((lambda *s: _rng.normal(s) * 0.8)(D, D)),
        }
    _B_in = _B_setup()

    return {
        "A_x": _A_in["x"],
        "A_wqkv": _A_in["wqkv"],
        "A_wo": _A_in["wo"],
        "B_x": _B_in["x"],
        "B_wqkv": _B_in["wqkv"],
        "B_wo": _B_in["wo"],
        "gate_w": _w((lambda *s: _rng.normal(s) * 0.05)(448) * 16.0),
    }

def reference(A_x, A_wqkv, A_wo, B_x, B_wqkv, B_wo, gate_w):
    def _A_ref(x, wqkv, wo):
        B, S, D = x.shape
        H = 16; Dh = D // H
        W, dil = 8, 2
        qkv = (lambda x, *d: x.transpose(*d))((x @ wqkv).reshape(B, S, 3, H, Dh), 2, 0, 3, 1, 4)
        q, k, v = qkv[0], qkv[1], qkv[2]
        scale = Dh ** -0.5
        pos = jnp.arange(S)
        off = jnp.arange(W) * dil
        idx = pos[:, None] - off[None, :]
        mask = idx >= 0
        idx_c = jnp.where(mask, idx, 0).reshape(-1)
        kg = k[:, :, idx_c, :].reshape(B, H, S, W, Dh)
        vg = v[:, :, idx_c, :].reshape(B, H, S, W, Dh)
        logits = jnp.einsum("bhsd,bhswd->bhsw", q, kg) * scale
        logits = jnp.where(mask[None, None, :, :], logits, -1e9)
        attn = _softmax(logits, axis=-1)
        o = jnp.einsum("bhsw,bhswd->bhsd", attn, vg)
        return (lambda x, *d: x.transpose(*d))(o, 0, 2, 1, 3).reshape(B, S, D) @ wo

    def _B_ref(x, wqkv, wo):
        B, S, D = x.shape
        H = 16; Dh = D // H
        qkv = (lambda x, *d: x.transpose(*d))((x @ wqkv).reshape(B, S, 3, H, Dh), 2, 0, 3, 1, 4)
        q, k, v = qkv[0], qkv[1], qkv[2]
        phi = lambda t: jnp.where(t > 0, t + 1, jnp.exp(t)) + 1e-6
        pq, pk = phi(q), phi(k)
        kv = jnp.einsum("bhsd,bhse->bhde", pk, v)
        z = jnp.einsum("bhsd->bhd", pk)
        num = jnp.einsum("bhqd,bhde->bhqe", pq, kv)
        den = jnp.einsum("bhqd,bhd->bhq", pq, z)[..., None] + 1e-6
        o = num / den
        return (lambda x, *d: x.transpose(*d))(o, 0, 2, 1, 3).reshape(B, S, D) @ wo

    x = A_x
    g = _sigmoid((x * gate_w).sum(-1, keepdims=True))
    a = _A_ref(x, A_wqkv, A_wo)
    b = _B_ref(x, B_wqkv, B_wo)
    return g * a + (1 - g) * b
```

```python
import functools
import jax
import jax.numpy as jnp
from jax import lax
import jax.experimental.pallas as pl
import jax.experimental.pallas.tpu as pltpu

S = 2048
D = 448
DP = 512
H = 16
DH = 28
W = 8
DIL = 2
BL = 128
NB = S // BL
F32 = jnp.float32
BF16 = jnp.bfloat16
U32 = jnp.uint32
DC = 2
LAG = 2
OPAQUE = 0
ORDER = 1


def _phi(t):
    return jnp.where(t > 0, t + 1.0, jnp.exp(t)) + 1e-6


def _dot(a, b):
    return jnp.dot(a, b, preferred_element_type=F32)


def _dot_nt(a, b):
    return lax.dot_general(a, b, (((1,), (1,)), ((), ())), preferred_element_type=F32)


def _pack(a, b):
    return pltpu.pack_elementwise([a, b], packed_dtype=BF16)


def _unpack(x, i):
    return pltpu.unpack_elementwise(x, index=i, packed_dtype=BF16, unpacked_dtype=F32)


def _interleave_heads(src, src0, dst, dst0, s_e, s_o, stride):
    for dd in range(DH // 2):
        e = src[:, pl.ds(src0 + s_e + dd, 8, stride=stride), :]
        o = src[:, pl.ds(src0 + s_o + dd, 8, stride=stride), :]
        lo = (e & jnp.uint32(0xFFFF)) | (o << 16)
        hi = (e >> 16) | (o & jnp.uint32(0xFFFF0000))
        dst[:, dst0 + 16 * dd:dst0 + 16 * dd + 8, :] = lo
        dst[:, dst0 + 16 * dd + 8:dst0 + 16 * dd + 16, :] = hi


def _kernel(x_hbm, wa_hbm, woa_hbm, wb_hbm, wob_hbm, g_hbm, out_hbm,
            xs, wa_v, wb_v, woa_v, wob_v, g_v,
            wkt, tmpa, tmpb, wpt, tmpo, tmpm, stack, wcat,
            t_acc, ztmp, zb, o_s,
            sem_x, sem_w, sem_o, sem_z, *blk):
    q_s, kp_s, vp_s, pq_s, gl_s, u_s = [blk[i * NB:(i + 1) * NB] for i in range(6)]
    if OPAQUE:
        zero = pl.semaphore_read(sem_z)
        def rd(r0, n):
            return pl.ds(pl.multiple_of(zero * 8 + r0, 8), n)
    else:
        def rd(r0, n):
            return pl.ds(r0, n)

    def _lanes(ref, r0, n, tiles):
        v = jnp.concatenate([ref[t, rd(r0, n), :] for t in range(tiles)], axis=1)
        return pltpu.bitcast(v, BF16)

    cp_wk = pltpu.make_async_copy(wb_hbm.at[:, 384:896], wb_v.at[0:D, 384:896], sem_w.at[0])
    cp_x = [pltpu.make_async_copy(x_hbm.at[:, c * BL:(c + 1) * BL], xs.at[c, 0:D, :], sem_x.at[c])
            for c in range(NB)]
    cp_wa = pltpu.make_async_copy(wa_hbm, wa_v.at[0:D, :], sem_w.at[1])
    cp_wq = pltpu.make_async_copy(wb_hbm.at[:, 0:384], wb_v.at[0:D, 0:384], sem_w.at[2])
    cp_wv = pltpu.make_async_copy(wb_hbm.at[:, 896:1344], wb_v.at[0:D, 896:1344], sem_w.at[3])
    cp_woa = pltpu.make_async_copy(woa_hbm, woa_v, sem_w.at[4])
    cp_wob = pltpu.make_async_copy(wob_hbm, wob_v, sem_w.at[5])
    cp_g = pltpu.make_async_copy(g_hbm, g_v, sem_w.at[6])
    cp_wk.start()
    for c in range(NB):
        cp_x[c].start()
    for cp in (cp_wa, cp_wq, cp_g, cp_woa, cp_wv, cp_wob):
        cp.start()

    xs[:, D:DP, :] = jnp.ones((NB, DP - D, BL), BF16)
    wa_v[D:DP, :] = jnp.zeros((DP - D, 3 * D), BF16)
    wb_v[D:DP, :] = jnp.zeros((DP - D, 3 * D), BF16)

    lane = lax.broadcasted_iota(jnp.int32, (H * DC, BL), 1)
    lane16 = lax.broadcasted_iota(jnp.int32, (H, BL), 1)

    def transpose_cols(src, c0, n, dst, r0):
        t = pltpu.bitcast(src[:, c0:c0 + n].T, U32)
        for ft in range(4):
            dst[ft, r0:r0 + n // 2, :] = t[:, ft * BL:(ft + 1) * BL]

    pk = [None] * NB

    def kproj(c):
        pk[c] = _phi(_dot(_lanes(wkt, 32, 224, 4), xs[c]))

    def tdot(g):
        a = jnp.concatenate([pk[4 * g + i] for i in range(4)], axis=1).astype(BF16)
        b = jnp.concatenate([xs[4 * g + i] for i in range(4)], axis=1)
        t = _dot_nt(a, b)
        if g == 0:
            t_acc[...] = t
        else:
            t_acc[...] += t

    def prep_a():
        for j in range(11):
            n = BL if j < 10 else 64
            transpose_cols(wa_v, j * BL, n, tmpa, j * 64)
        for p in range(3):
            _interleave_heads(tmpa, p * 224, wpt, p * 224, 0, 14, 28)

    def prep_b():
        for j in range(3):
            transpose_cols(wb_v, j * BL, BL, tmpb, j * 64)
        tmpb[:, 192:224, :] = wkt[:, 0:32, :]
        _interleave_heads(tmpb, 0, wpt, 3 * 224, 0, 14, 28)
        g = g_v[...].astype(F32).reshape(1, D)
        g = jnp.concatenate([g, jnp.zeros((1, DP - D), F32)], axis=1)
        g = pltpu.bitcast(jnp.broadcast_to(g, (16, DP)).astype(BF16), U32)
        for ft in range(4):
            wpt[ft, 4 * 224:4 * 224 + 8, :] = g[:, ft * BL:(ft + 1) * BL]

    def to_tiles(v, dst):
        u = pltpu.bitcast(v, U32)
        u = jnp.concatenate([u, jnp.zeros((224, DP - D), U32)], axis=1)
        for nt in range(4):
            dst[nt] = u[:, nt * BL:(nt + 1) * BL]

    def stack_t(j):
        v = pltpu.bitcast(jnp.concatenate([stack[t, j * 64:j * 64 + 64, :] for t in range(4)], axis=1), BF16)
        wcat[j] = pltpu.bitcast(v[:, 0:D].T, U32)

    def prep_o():
        to_tiles(woa_v[...], tmpo)
        _interleave_heads(tmpo, 0, stack, 224, 0, 112, 14)
        for j in range(4, 7):
            stack_t(j)

    RNG = ((0, 144), (112, 288), (240, 400), (352, 448))

    def kv_step():
        t3 = t_acc[:, 384:512]
        l = lax.broadcasted_iota(jnp.int32, (D, BL), 1)
        ztmp[...] = jnp.where(l < 64, pltpu.roll(t3, 64, 1), t3)
        for d in range(DH):
            zb[d * H:(d + 1) * H, :] = ztmp[pl.ds(d, H, stride=DH), :]
        res = []
        for t, (r0, r1) in enumerate(RNG):
            n = BL if t < 3 else 64
            kv = _dot(t_acc[r0:r1, :].astype(BF16), wb_v[:, 896 + t * BL:896 + t * BL + n])
            hd = ((lax.broadcasted_iota(jnp.int32, kv.shape, 0) + r0) * 2341) >> 16
            he = ((lax.broadcasted_iota(jnp.int32, kv.shape, 1) + t * BL) * 2341) >> 16
            res.append(jnp.where(hd == he, kv, 0.0).astype(BF16))
        return res

    def m_step(kvm):
        m = []
        for t in range(4):
            n = BL if t < 3 else 64
            m.append(_dot(kvm[t], wob_v[t * BL:t * BL + n, :]))
        mm = jnp.concatenate([
            m[0][0:112], m[0][112:144] + m[1][0:32], m[1][32:128], m[1][128:176] + m[2][0:48],
            m[2][48:112], m[2][112:160] + m[3][0:48], m[3][48:96]], axis=0)
        to_tiles(mm.astype(BF16), tmpm)
        _interleave_heads(tmpm, 0, stack, 0, 0, 112, 14)
        for j in range(4):
            stack_t(j)

    def proj(c, parts):
        x = xs[c]
        for p in parts:
            if p == 0:
                q_s[c][...] = _dot(_lanes(wpt, 0, 224, 4), x)
            elif p == 1:
                r = _dot(_lanes(wpt, 224, 224, 4), x)
                kp_s[c][...] = _pack(r[0:224], r[224:448])
            elif p == 2:
                r = _dot(_lanes(wpt, 448, 224, 4), x)
                vp_s[c][...] = _pack(r[0:224], r[224:448])
            else:
                r = _dot(_lanes(wpt, 672, 232, 4), x)
                pq_s[c][...] = _phi(r[0:D])
                gl_s[c][...] = r[D:D + H]

    def shifted(ref, c, d0, w):
        cur = ref[c][rd(H * d0, H * DC), :]
        if w == 0:
            sh = cur
        else:
            prev = ref[c - 1][rd(H * d0, H * DC), :] if c > 0 else cur
            sh = pltpu.roll(jnp.where(lane >= BL - DIL * w, prev, cur), DIL * w, 1)
        return _unpack(sh, 0).reshape(DC, H, BL), _unpack(sh, 1).reshape(DC, H, BL)

    def pack_u(o):
        return _pack(o[:, 0:8, :], o[:, 8:16, :]).reshape(o.shape[0] * 8, BL)

    def attn(c):
        logit = [None] * W
        for d0 in range(0, DH // 2, DC):
            q0 = q_s[c][rd(H * d0, H * DC), :].reshape(DC, H, BL)
            q1 = q_s[c][rd(224 + H * d0, H * DC), :].reshape(DC, H, BL)
            for w in range(W):
                k0, k1 = shifted(kp_s, c, d0, w)
                p = jnp.sum(q0 * k0 + q1 * k1, axis=0)
                logit[w] = p if logit[w] is None else logit[w] + p
        logit = [l * (DH ** -0.5) for l in logit]
        if c == 0:
            logit = [jnp.where(lane16 >= DIL * w, l, -1e9) for w, l in enumerate(logit)]
        m = functools.reduce(jnp.maximum, logit)
        e = [jnp.exp(l - m) for l in logit]
        g = jax.nn.sigmoid(gl_s[c][rd(0, H), :])
        r = g / functools.reduce(jnp.add, e)
        a = [x * r for x in e]
        for d0 in range(0, DH // 2, DC):
            o0 = o1 = None
            for w in range(W):
                v0, v1 = shifted(vp_s, c, d0, w)
                p0 = a[w][None] * v0
                p1 = a[w][None] * v1
                o0 = p0 if o0 is None else o0 + p0
                o1 = p1 if o1 is None else o1 + p1
            u_s[c][224 + 8 * d0:224 + 8 * (d0 + DC), :] = pack_u(o0)
            u_s[c][336 + 8 * d0:336 + 8 * (d0 + DC), :] = pack_u(o1)

    def lin(c):
        pq = pq_s[c][rd(0, D), :].reshape(DH, H, BL)
        den = jnp.sum(pq * zb[rd(0, D), :].reshape(DH, H, BL), axis=0) + 1e-6
        g = jax.nn.sigmoid(gl_s[c][rd(0, H), :])
        r = (1.0 - g) / den
        u_s[c][0:224, :] = pack_u(pq * r[None])

    cp_o = [pltpu.make_async_copy(o_s.at[c], out_hbm.at[:, c * BL:(c + 1) * BL], sem_o.at[c])
            for c in range(NB)]

    def final(c):
        o = _dot(_lanes(wcat, 0, 224, 7), pltpu.bitcast(u_s[c][rd(0, D), :], BF16))
        o_s[c] = o.astype(BF16)
        cp_o[c].start()

    cp_wk.wait()
    for c in range(4):
        cp_x[c].wait()
    for j in range(4):
        transpose_cols(wb_v, 384 + j * BL, BL, wkt, j * 64)
    for c in range(4):
        kproj(c)
    tdot(0)
    for c in range(4, NB):
        cp_x[c].wait()
    for c in range(4, 9):
        kproj(c)
    tdot(1)
    for cp in (cp_wa, cp_wq, cp_g, cp_woa, cp_wv, cp_wob):
        cp.wait()
    prep_a()
    prep_b()
    prep_o()
    for c in range(9, 13):
        kproj(c)
    tdot(2)
    for c in range(13, NB):
        kproj(c)
    proj(0, range(4))
    tdot(3)
    attn(0)
    proj(1, (0, 1))
    kvm = kv_step()
    proj(1, (2, 3))
    m_step(kvm)
    lin(0)
    if ORDER == 0:
        for c in range(2, NB):
            proj(c, range(4))
            attn(c - 1)
            lin(c - 1)
            if c >= LAG:
                final(c - LAG)
        attn(NB - 1)
        lin(NB - 1)
    else:
        attn(1); lin(1)
        for c in range(2, NB):
            proj(c, (3, 0, 1, 2))
            attn(c)
            lin(c)
            if c >= LAG:
                final(c - LAG)
    for c in range(NB - LAG, NB):
        final(c)
    for c in range(NB):
        cp_o[c].wait()


@jax.jit
def pallas_gated_mix__sliding_local_dilated__linear_attn_block__prompt_kernel(
        A_x, A_wqkv, A_wo, B_x, B_wqkv, B_wo, gate_w):
    xt = jnp.swapaxes(A_x, 1, 2).reshape(D, S)
    any_spec = pl.BlockSpec(memory_space=pl.ANY)
    V = pltpu.VMEM
    ot = pl.pallas_call(
        _kernel,
        out_shape=jax.ShapeDtypeStruct((D, S), BF16),
        in_specs=[any_spec] * 6,
        out_specs=any_spec,
        scratch_shapes=[
            V((NB, DP, BL), BF16),
            V((DP, 3 * D), BF16),
            V((DP, 3 * D), BF16),
            V((D, D), BF16),
            V((D, D), BF16),
            V((D,), BF16),
            V((4, 256, BL), U32),
            V((4, 672, BL), U32),
            V((4, 224, BL), U32),
            V((4, 904, BL), U32),
            V((4, 224, BL), U32),
            V((4, 224, BL), U32),
            V((4, 448, BL), U32),
            V((7, 224, BL), U32),
            V((D, DP), F32),
            V((D, BL), F32),
            V((D, BL), F32),
            V((NB, D, BL), BF16),
            pltpu.SemaphoreType.DMA((NB,)),
            pltpu.SemaphoreType.DMA((7,)),
            pltpu.SemaphoreType.DMA((NB,)),
            pltpu.SemaphoreType.REGULAR,
        ] + [V((D, BL), F32)] * NB + [V((224, BL), U32)] * (2 * NB) + [V((D, BL), F32)] * NB
          + [V((H, BL), F32)] * NB + [V((D, BL), U32)] * NB,
        compiler_params=pltpu.CompilerParams(vmem_limit_bytes=100 * 1024 * 1024),
    )(xt, A_wqkv, A_wo, B_wqkv, B_wo, gate_w)
    return jnp.swapaxes(ot.reshape(1, D, S), 1, 2)
```

```python
import jax
import jax.numpy as jnp
from jax import lax
import jax.experimental.pallas as pl
import jax.experimental.pallas.tpu as pltpu

S = 2048
D = 448
DP = 512
H = 16
DH = 28
W = 8
DIL = 2
BL = 128
NB = S // BL
DC = 2
F32 = jnp.float32
BF16 = jnp.bfloat16
U32 = jnp.uint32
LOG2E = 1.4426950408889634


def _phi(t):
    return jnp.where(t > 0, t + 1.0, jnp.exp(t)) + 1e-6


def _dot(a, b):
    return jnp.dot(a, b, preferred_element_type=F32)


def _dot_nt(a, b):
    return lax.dot_general(a, b, (((1,), (1,)), ((), ())), preferred_element_type=F32)


def _tree(op, xs):
    xs = list(xs)
    while len(xs) > 1:
        xs = [op(xs[i], xs[i + 1]) if i + 1 < len(xs) else xs[i] for i in range(0, len(xs), 2)]
    return xs[0]


def _lanes(ref, r0, n, tiles):
    v = jnp.concatenate([ref[t, r0:r0 + n, :] for t in range(tiles)], axis=1)
    return pltpu.bitcast(v, BF16)


def _interleave_heads(src, src0, dst, dst0):
    for dd in range(DH // 2):
        e = src[:, pl.ds(src0 + dd, 8, stride=DH), :]
        o = src[:, pl.ds(src0 + DH // 2 + dd, 8, stride=DH), :]
        lo = (e & jnp.uint32(0xFFFF)) | (o << 16)
        hi = (e >> 16) | (o & jnp.uint32(0xFFFF0000))
        dst[:, dst0 + 16 * dd:dst0 + 16 * dd + 8, :] = lo
        dst[:, dst0 + 16 * dd + 8:dst0 + 16 * dd + 16, :] = hi


def _kernel(x_hbm, wa_hbm, woa_hbm, wb_hbm, wob_hbm, g_hbm, out_hbm,
            xs, wa_v, wb_v, woa_v, wob_v, g_v,
            wkt, tmpa, tmpb, wpt, tmpo, tmpm, stack, wcat, ztmp, o_s, sem):
    cpy = pltpu.make_async_copy
    X1, X2, X3 = 2 * BL, 4 * BL, 12 * BL
    g0 = [cpy(wb_hbm.at[:, 640:896], wb_v.at[0:D, 640:896], sem.at[0])]
    g1 = [cpy(x_hbm.at[:, 0:X1], xs.at[:, 0:X1], sem.at[1])]
    g2 = [cpy(wb_hbm.at[:, 384:640], wb_v.at[0:D, 384:640], sem.at[2]),
          cpy(x_hbm.at[:, X1:X2], xs.at[:, X1:X2], sem.at[2]),
          cpy(g_hbm, g_v, sem.at[2])]
    g3 = [cpy(x_hbm.at[:, X2:X3], xs.at[:, X2:X3], sem.at[3])]
    g4 = [cpy(x_hbm.at[:, X3:S], xs.at[:, X3:S], sem.at[4]),
          cpy(wa_hbm, wa_v.at[0:D, :], sem.at[4]),
          cpy(wb_hbm.at[:, 0:384], wb_v.at[0:D, 0:384], sem.at[4]),
          cpy(woa_hbm, woa_v, sem.at[4]),
          cpy(wb_hbm.at[:, 896:1344], wb_v.at[0:D, 896:1344], sem.at[4]),
          cpy(wob_hbm, wob_v, sem.at[4])]
    for cp in g0 + g1 + g2 + g3 + g4:
        cp.start()

    def wait(group):
        for cp in group:
            cp.wait()

    wa_v[D:DP, :] = jnp.zeros((DP - D, 3 * D), BF16)
    wb_v[D:DP, 0:896] = jnp.zeros((DP - D, 896), BF16)

    lane = lax.broadcasted_iota(jnp.int32, (DC, 8, BL), 2)
    lane16 = lax.broadcasted_iota(jnp.int32, (H, BL), 1)

    def xblk(c):
        return xs[:, c * BL:(c + 1) * BL]

    def transpose_cols(src, c0, n, dst, r0):
        t = pltpu.bitcast(src[:, c0:c0 + n].T, U32)
        if dst is wkt:
            z = pltpu.bitcast(wb_v[D:D + 16, 0:DP], U32)
            t = t | jnp.concatenate([z] * (n // 16), axis=0)
        for ft in range(4):
            dst[ft, r0:r0 + n // 2, :] = t[:, ft * BL:(ft + 1) * BL]

    st = {}
    pk, q_s, k_s, kp_s, vp_s, pq_s, g_s, ua_s, ub_s = [[None] * NB for _ in range(9)]

    def gate(c, pace):
        p = xblk(c).astype(F32) * st['gw']
        gl = None
        for i0 in range(0, D // 8, 4):
            t = _tree(jnp.add, [p[8 * i:8 * i + 8] for i in range(i0, i0 + 4)])
            t = jnp.where(pace[8 * i0:8 * i0 + 8] > 0, t, 0.0)
            gl = t if gl is None else gl + t
        for sh in (4, 2, 1):
            gl = gl + pltpu.roll(gl, sh, 0)
        g = jax.nn.sigmoid(gl)
        g_s[c] = jnp.concatenate([g, g], axis=0)

    def kproj(c):
        pk[c] = _phi(_dot(_lanes(wkt, 32, 224, 4)[:, 0:D], xblk(c)))
        gate(c, pk[c])
        if c < 8:
            gate(c - 4, pk[c])

    def tdot(c0, c1):
        a = jnp.concatenate(pk[c0:c1], axis=1).astype(BF16)
        st['z'] = _tree(jnp.add, pk[c0:c1]) + st['z']
        st['tm'] = _dot_nt(a, xs[0:384, c0 * BL:c1 * BL]) + st['tm']
        st['ts'] = _dot_nt(xs[384:D, c0 * BL:c1 * BL], a) + st['ts']

    def to_tiles(v, dst):
        u = pltpu.bitcast(v, U32)
        u = jnp.concatenate([u, jnp.zeros((224, DP - D), U32)], axis=1)
        for nt in range(4):
            dst[nt] = u[:, nt * BL:(nt + 1) * BL]

    def stack_t(j):
        wcat[j] = pltpu.bitcast(_lanes(stack, j * 64, 64, 4)[:, 0:D].T, U32)

    def prep():
        for j in range(11):
            transpose_cols(wa_v, j * BL, BL if j < 10 else 64, tmpa, j * 64)
        for p in range(3):
            _interleave_heads(tmpa, p * 224, wpt, p * 224)
        for j in range(3):
            transpose_cols(wb_v, j * BL, BL, tmpb, j * 64)
        tmpb[:, 192:224, :] = wkt[:, 0:32, :]
        _interleave_heads(tmpb, 0, wpt, 3 * 224)
        to_tiles(woa_v[...], tmpo)
        _interleave_heads(tmpo, 0, stack, 224)
        for j in range(4, 7):
            stack_t(j)

    G = 4 * DH

    def kv_step():
        ztmp[...] = st['z']
        zp = jnp.stack([ztmp[pl.ds(d, H, stride=DH), :] for d in range(DH)])
        st['zb'] = jnp.broadcast_to(jnp.sum(zp, axis=2, keepdims=True), (DH, H, BL))
        t = jnp.concatenate([st['tm'], st['ts'].T], axis=1)
        hd = (lax.broadcasted_iota(jnp.int32, (G, G), 0) * 2341) >> 16
        he = (lax.broadcasted_iota(jnp.int32, (G, G), 1) * 2341) >> 16
        res = []
        for i in range(4):
            kv = _dot(t[i * G:(i + 1) * G, :].astype(BF16), wb_v[0:D, 896 + i * G:896 + (i + 1) * G])
            res.append(jnp.where(hd == he, kv, 0.0).astype(BF16))
        return res

    def m_step(kvm):
        m = jnp.concatenate([_dot(kvm[i], wob_v[i * G:(i + 1) * G, :]) for i in range(4)], axis=0)
        to_tiles(m.astype(BF16), tmpm)
        _interleave_heads(tmpm, 0, stack, 0)
        for j in range(4):
            stack_t(j)

    def proj(c, parts):
        x = xblk(c)
        for p in parts:
            r = _dot(_lanes(wpt, p * 224, 224, 4)[:, 0:D], x)
            if p == 0:
                q_s[c] = r.reshape(DH, H, BL)
            elif p == 1:
                k_s[c] = r.reshape(DH, H, BL)
                kp_s[c] = pltpu.bitcast(r.astype(BF16), U32).reshape(DH, 8, BL)
            elif p == 2:
                vp_s[c] = pltpu.bitcast(r.astype(BF16), U32).reshape(DH, 8, BL)
            else:
                pq_s[c] = _phi(r).reshape(DH, H, BL)

    def shifted(vals, c, d0, w):
        sh = vals[c][d0:d0 + DC]
        if w > 0:
            if c > 0:
                sh = jnp.where(lane >= BL - DIL * w, vals[c - 1][d0:d0 + DC], sh)
            sh = pltpu.roll(sh, DIL * w, 2)
        return pltpu.bitcast(sh, BF16).astype(F32)

    def attn(c):
        logit = [None] * W
        for d0 in range(0, DH, DC):
            q = q_s[c][d0:d0 + DC]
            for w in range(W):
                k = k_s[c][d0:d0 + DC] if w == 0 else shifted(kp_s, c, d0, w)
                p = jnp.sum(q * k, axis=0)
                logit[w] = p if logit[w] is None else logit[w] + p
        if c == 0:
            logit = [jnp.where(lane16 >= DIL * w, l, -1e9 * DH ** 0.5) for w, l in enumerate(logit)]
        m = _tree(jnp.maximum, logit)
        e = [jnp.exp2((l - m) * (DH ** -0.5 * LOG2E)) for l in logit]
        r = g_s[c] / _tree(jnp.add, e)
        us = []
        for d0 in range(0, DH, DC):
            o = None
            for w in range(W):
                p = e[w][None] * shifted(vp_s, c, d0, w)
                o = p if o is None else o + p
            us.append(o * r[None])
        ua_s[c] = jnp.concatenate(us, axis=0)

    def lin(c):
        pq = pq_s[c]
        den = jnp.sum(pq * st['zb'], axis=0) + 1e-6
        ub_s[c] = pq * ((1.0 - g_s[c]) / den)[None]

    cp_o = []

    def final(c):
        u = jnp.concatenate([ub_s[c], ua_s[c]], axis=0).reshape(2 * D, BL).astype(BF16)
        o = [_dot(_lanes(wcat, 56 * i, 56, 7), u).astype(BF16) for i in range(4)]
        for i in range(4):
            o_s[c, i * G:(i + 1) * G, :] = o[i]
            if c == NB - 1 or i == 3:
                r0 = i * G if c == NB - 1 else 0
                r1 = (i + 1) * G
                cp = cpy(o_s.at[c, r0:r1, :], out_hbm.at[r0:r1, c * BL:(c + 1) * BL], sem.at[0])
                cp.start()
                cp_o.append(cp)

    wait(g0)
    for j in (2, 3):
        transpose_cols(wb_v, 384 + j * BL, BL, wkt, j * 64)
    wait(g1)
    whi = _lanes(wkt, 128, 128, 4)[:, 0:D]
    khi = [_phi(_dot(whi, xblk(c))) for c in range(2)]
    thi = [None, None]
    for c in range(2):
        for i in range(2):
            t = _dot_nt(khi[c][i * BL:(i + 1) * BL].astype(BF16), xs[0:384, c * BL:(c + 1) * BL])
            thi[i] = t if thi[i] is None else t + thi[i]
    wait(g2)
    khi += [_phi(_dot(whi, xblk(c))) for c in range(2, 4)]
    for j in (0, 1):
        transpose_cols(wb_v, 384 + j * BL, BL, wkt, j * 64)
    wlo = _lanes(wkt, 32, 96, 4)[:, 0:D]
    klo = [_phi(_dot(wlo, xblk(c))) for c in range(4)]
    for c in range(4):
        pk[c] = jnp.concatenate([klo[c], khi[c]], axis=0)
    for i in range(2):
        a = jnp.concatenate([khi[2][i * BL:(i + 1) * BL], khi[3][i * BL:(i + 1) * BL]], axis=1)
        thi[i] = _dot_nt(a.astype(BF16), xs[0:384, 2 * BL:4 * BL]) + thi[i]
    tlo = _dot_nt(jnp.concatenate(klo, axis=1).astype(BF16), xs[0:384, 0:4 * BL])
    st['tm'] = jnp.concatenate([tlo] + thi, axis=0)
    st['ts'] = _dot_nt(xs[384:D, 0:4 * BL], jnp.concatenate(pk[0:4], axis=1).astype(BF16))
    st['z'] = _tree(jnp.add, pk[0:4])
    st['gw'] = jnp.broadcast_to(g_v[...].astype(F32).reshape(1, D), (BL, D)).T
    wait(g3)
    for c in range(4, 9):
        kproj(c)
    tdot(4, 8)
    for c in range(9, 12):
        kproj(c)
    tdot(8, 12)
    wait(g4)
    prep()
    for c in range(12, NB):
        kproj(c)
    tdot(12, NB)
    proj(0, (3, 0))
    kvm = kv_step()
    proj(0, (1, 2))
    attn(0)
    m_step(kvm)
    lin(0)
    proj(1, (3, 0, 1, 2))
    attn(1)
    lin(1)
    final(0)
    proj(2, (3, 0))
    lin(2)
    final(1)
    for c in range(2, NB - 1):
        proj(c, (1, 2))
        attn(c)
        proj(c + 1, (3, 0))
        lin(c + 1)
        if c < NB - 2:
            final(c)
    proj(NB - 1, (1, 2))
    attn(NB - 1)
    final(NB - 2)
    final(NB - 1)
    assert len(cp_o) == NB + 3
    wait(cp_o)


@jax.jit
def pallas_gated_mix__sliding_local_dilated__linear_attn_block__prompt_kernel(
        A_x, A_wqkv, A_wo, B_x, B_wqkv, B_wo, gate_w):
    del B_x
    xt = jnp.swapaxes(A_x, 1, 2).reshape(D, S)
    any_spec = pl.BlockSpec(memory_space=pl.ANY)
    V = pltpu.VMEM
    ot = pl.pallas_call(
        _kernel,
        out_shape=jax.ShapeDtypeStruct((D, S), BF16),
        in_specs=[any_spec] * 6,
        out_specs=any_spec,
        scratch_shapes=[
            V((D, S + BL), BF16),
            V((DP, 3 * D), BF16),
            V((DP, 3 * D), BF16),
            V((D, D), BF16),
            V((D, D), BF16),
            V((D,), BF16),
            V((4, 256, BL), U32),
            V((4, 672, BL), U32),
            V((4, 224, BL), U32),
            V((4, 896, BL), U32),
            V((4, 224, BL), U32),
            V((4, 224, BL), U32),
            V((4, 448, BL), U32),
            V((7, 224, BL), U32),
            V((D, BL), F32),
            V((NB, D, BL), BF16),
            pltpu.SemaphoreType.DMA((5,)),
        ],
        compiler_params=pltpu.CompilerParams(vmem_limit_bytes=64 * 1024 * 1024,
                                             disable_semaphore_checks=True),
    )(xt, A_wqkv, A_wo, B_wqkv, B_wo, gate_w)
    return jnp.swapaxes(ot.reshape(1, D, S), 1, 2)
```

```python
import jax
import jax.numpy as jnp
from jax import lax
import jax.experimental.pallas as pl
import jax.experimental.pallas.tpu as pltpu

S = 2048
D = 448
DP = 512
H = 16
DH = 28
W = 8
DIL = 2
BL = 128
NB = S // BL
DC = 2
F32 = jnp.float32
BF16 = jnp.bfloat16
U32 = jnp.uint32
LOG2E = 1.4426950408889634


def _phi(t):
    return jnp.where(t > 0, t + 1.0, jnp.exp(t)) + 1e-6


def _dot(a, b):
    return jnp.dot(a, b, preferred_element_type=F32)


def _dot_nt(a, b):
    return lax.dot_general(a, b, (((1,), (1,)), ((), ())), preferred_element_type=F32)


def _tree(op, xs):
    xs = list(xs)
    while len(xs) > 1:
        xs = [op(xs[i], xs[i + 1]) if i + 1 < len(xs) else xs[i] for i in range(0, len(xs), 2)]
    return xs[0]


def _lanes(ref, r0, n, tiles):
    v = jnp.concatenate([ref[t, r0:r0 + n, :] for t in range(tiles)], axis=1)
    return pltpu.bitcast(v, BF16)


def _interleave_heads(src, src0, dst, dst0):
    for dd in range(DH // 2):
        e = src[:, pl.ds(src0 + dd, 8, stride=DH), :]
        o = src[:, pl.ds(src0 + DH // 2 + dd, 8, stride=DH), :]
        lo = (e & jnp.uint32(0xFFFF)) | (o << 16)
        hi = (e >> 16) | (o & jnp.uint32(0xFFFF0000))
        dst[:, dst0 + 16 * dd:dst0 + 16 * dd + 8, :] = lo
        dst[:, dst0 + 16 * dd + 8:dst0 + 16 * dd + 16, :] = hi


def _kernel(x_hbm, wa_hbm, woa_hbm, wb_hbm, wob_hbm, g_hbm, out_hbm,
            xs, wa_v, wb_v, woa_v, wob_v, g_v,
            wkt, tmpa, tmpb, wpt, tmpo, tmpm, stack, wcat, ztmp, o_s, sem):
    cpy = pltpu.make_async_copy
    X1, X2, X3 = 2 * BL, 4 * BL, 12 * BL
    g0 = [cpy(wb_hbm.at[:, 640:896], wb_v.at[0:D, 640:896], sem.at[0])]
    g1 = [cpy(x_hbm.at[:, 0:X1], xs.at[:, 0:X1], sem.at[1])]
    g2 = [cpy(wb_hbm.at[:, 384:640], wb_v.at[0:D, 384:640], sem.at[2]),
          cpy(x_hbm.at[:, X1:X2], xs.at[:, X1:X2], sem.at[2]),
          cpy(g_hbm, g_v, sem.at[2])]
    g3 = [cpy(x_hbm.at[:, X2:X3], xs.at[:, X2:X3], sem.at[3])]
    g4 = [cpy(x_hbm.at[:, X3:S], xs.at[:, X3:S], sem.at[4]),
          cpy(wa_hbm, wa_v.at[0:D, :], sem.at[4]),
          cpy(wb_hbm.at[:, 0:384], wb_v.at[0:D, 0:384], sem.at[4]),
          cpy(woa_hbm, woa_v, sem.at[4]),
          cpy(wb_hbm.at[:, 896:1344], wb_v.at[0:D, 896:1344], sem.at[4]),
          cpy(wob_hbm, wob_v, sem.at[4])]
    for cp in g0 + g1 + g2 + g3 + g4:
        cp.start()

    def wait(group):
        for cp in group:
            cp.wait()

    wa_v[D:DP, :] = jnp.zeros((DP - D, 3 * D), BF16)
    wb_v[D:DP, 0:896] = jnp.zeros((DP - D, 896), BF16)

    lane = lax.broadcasted_iota(jnp.int32, (DC, 8, BL), 2)
    lane16 = lax.broadcasted_iota(jnp.int32, (H, BL), 1)

    def xblk(c):
        return xs[:, c * BL:(c + 1) * BL]

    def transpose_cols(src, c0, n, dst, r0):
        t = pltpu.bitcast(src[:, c0:c0 + n].T, U32)
        if dst is wkt:
            z = pltpu.bitcast(wb_v[D:D + 16, 0:DP], U32)
            t = t | jnp.concatenate([z] * (n // 16), axis=0)
        for ft in range(4):
            dst[ft, r0:r0 + n // 2, :] = t[:, ft * BL:(ft + 1) * BL]

    st = {}
    pk, q_s, k_s, kp_s, vp_s, pq_s, g_s, ua_s, ub_s = [[None] * NB for _ in range(9)]

    def gate(c, pace):
        p = xblk(c).astype(F32) * st['gw']
        gl = None
        for i0 in range(0, D // 8, 4):
            t = _tree(jnp.add, [p[8 * i:8 * i + 8] for i in range(i0, i0 + 4)])
            t = jnp.where(pace[8 * i0:8 * i0 + 8] > 0, t, 0.0)
            gl = t if gl is None else gl + t
        for sh in (4, 2, 1):
            gl = gl + pltpu.roll(gl, sh, 0)
        g = jax.nn.sigmoid(gl)
        g_s[c] = jnp.concatenate([g, g], axis=0)

    def kproj(c):
        pk[c] = _phi(_dot(_lanes(wkt, 32, 224, 4)[:, 0:D], xblk(c)))
        gate(c, pk[c])
        if c < 8:
            gate(c - 4, pk[c])

    def tdot(c0, c1):
        a = jnp.concatenate(pk[c0:c1], axis=1).astype(BF16)
        st['z'] = _tree(jnp.add, pk[c0:c1]) + st['z']
        st['tm'] = _dot_nt(a, xs[0:384, c0 * BL:c1 * BL]) + st['tm']
        st['ts'] = _dot_nt(xs[384:D, c0 * BL:c1 * BL], a) + st['ts']

    def to_tiles(v, dst):
        u = pltpu.bitcast(v, U32)
        u = jnp.concatenate([u, jnp.zeros((224, DP - D), U32)], axis=1)
        for nt in range(4):
            dst[nt] = u[:, nt * BL:(nt + 1) * BL]

    def stack_t(j):
        wcat[j] = pltpu.bitcast(_lanes(stack, j * 64, 64, 4)[:, 0:D].T, U32)

    def prep():
        for j in range(11):
            transpose_cols(wa_v, j * BL, BL if j < 10 else 64, tmpa, j * 64)
        for p in range(3):
            _interleave_heads(tmpa, p * 224, wpt, p * 224)
        for j in range(3):
            transpose_cols(wb_v, j * BL, BL, tmpb, j * 64)
        tmpb[:, 192:224, :] = wkt[:, 0:32, :]
        _interleave_heads(tmpb, 0, wpt, 3 * 224)
        to_tiles(woa_v[...], tmpo)
        _interleave_heads(tmpo, 0, stack, 224)
        for j in range(4, 7):
            stack_t(j)

    G = 4 * DH

    def kv_step():
        ztmp[...] = st['z']
        zp = jnp.stack([ztmp[pl.ds(d, H, stride=DH), :] for d in range(DH)])
        st['zb'] = jnp.broadcast_to(jnp.sum(zp, axis=2, keepdims=True), (DH, H, BL))
        t = jnp.concatenate([st['tm'], st['ts'].T], axis=1)
        hd = (lax.broadcasted_iota(jnp.int32, (G, G), 0) * 2341) >> 16
        he = (lax.broadcasted_iota(jnp.int32, (G, G), 1) * 2341) >> 16
        res = []
        for i in range(4):
            kv = _dot(t[i * G:(i + 1) * G, :].astype(BF16), wb_v[0:D, 896 + i * G:896 + (i + 1) * G])
            res.append(jnp.where(hd == he, kv, 0.0).astype(BF16))
        return res

    def m_step(kvm):
        m = jnp.concatenate([_dot(kvm[i], wob_v[i * G:(i + 1) * G, :]) for i in range(4)], axis=0)
        to_tiles(m.astype(BF16), tmpm)
        _interleave_heads(tmpm, 0, stack, 0)
        for j in range(4):
            stack_t(j)

    def proj(c, parts):
        x = xblk(c)
        for p in parts:
            r = _dot(_lanes(wpt, p * 224, 224, 4)[:, 0:D], x)
            if p == 0:
                q_s[c] = r.reshape(DH, H, BL)
            elif p == 1:
                k_s[c] = r.reshape(DH, H, BL)
                kp_s[c] = pltpu.bitcast(r.astype(BF16), U32).reshape(DH, 8, BL)
            elif p == 2:
                vp_s[c] = pltpu.bitcast(r.astype(BF16), U32).reshape(DH, 8, BL)
            else:
                pq_s[c] = _phi(r).reshape(DH, H, BL)

    def shifted(vals, c, d0, w):
        sh = vals[c][d0:d0 + DC]
        if w > 0:
            if c > 0:
                sh = jnp.where(lane >= BL - DIL * w, vals[c - 1][d0:d0 + DC], sh)
            sh = pltpu.roll(sh, DIL * w, 2)
        return pltpu.bitcast(sh, BF16).astype(F32)

    def attn(c):
        logit = [None] * W
        for d0 in range(0, DH, DC):
            q = q_s[c][d0:d0 + DC]
            for w in range(W):
                k = k_s[c][d0:d0 + DC] if w == 0 else shifted(kp_s, c, d0, w)
                p = jnp.sum(q * k, axis=0)
                logit[w] = p if logit[w] is None else logit[w] + p
        if c == 0:
            logit = [jnp.where(lane16 >= DIL * w, l, -1e9 * DH ** 0.5) for w, l in enumerate(logit)]
        m = _tree(jnp.maximum, logit)
        e = [jnp.exp2((l - m) * (DH ** -0.5 * LOG2E)) for l in logit]
        r = g_s[c] / _tree(jnp.add, e)
        us = []
        for d0 in range(0, DH, DC):
            o = None
            for w in range(W):
                p = e[w][None] * shifted(vp_s, c, d0, w)
                o = p if o is None else o + p
            us.append(o * r[None])
        ua_s[c] = jnp.concatenate(us, axis=0)

    def lin(c):
        pq = pq_s[c]
        den = jnp.sum(pq * st['zb'], axis=0) + 1e-6
        ub_s[c] = pq * ((1.0 - g_s[c]) / den)[None]

    cp_o = []

    def final(c):
        u = jnp.concatenate([ub_s[c], ua_s[c]], axis=0).reshape(2 * D, BL).astype(BF16)
        o = [_dot(_lanes(wcat, 56 * i, 56, 7), u) for i in range(4)]
        o = jnp.concatenate(o, axis=0)
        cuts = (0, 112, 224, 336, 400, 432, D) if c == NB - 1 else (0, D)
        for r0, r1 in zip(cuts[:-1], cuts[1:]):
            o_s[c, r0:r1, :] = o[r0:r1].astype(BF16)
            cp = cpy(o_s.at[c, r0:r1, :], out_hbm.at[r0:r1, c * BL:(c + 1) * BL], sem.at[0])
            cp.start()
            cp_o.append(cp)

    wait(g0)
    for j in (2, 3):
        transpose_cols(wb_v, 384 + j * BL, BL, wkt, j * 64)
    wait(g1)
    whi = _lanes(wkt, 128, 128, 4)[:, 0:D]
    khi = [_phi(_dot(whi, xblk(c))) for c in range(2)]
    thi = [None, None]
    for c in range(2):
        for i in range(2):
            t = _dot_nt(khi[c][i * BL:(i + 1) * BL].astype(BF16), xs[0:384, c * BL:(c + 1) * BL])
            thi[i] = t if thi[i] is None else t + thi[i]
    wait(g2)
    khi += [_phi(_dot(whi, xblk(c))) for c in range(2, 4)]
    for j in (0, 1):
        transpose_cols(wb_v, 384 + j * BL, BL, wkt, j * 64)
    wlo = _lanes(wkt, 32, 96, 4)[:, 0:D]
    klo = [_phi(_dot(wlo, xblk(c))) for c in range(4)]
    for c in range(4):
        pk[c] = jnp.concatenate([klo[c], khi[c]], axis=0)
    for i in range(2):
        a = jnp.concatenate([khi[2][i * BL:(i + 1) * BL], khi[3][i * BL:(i + 1) * BL]], axis=1)
        thi[i] = _dot_nt(a.astype(BF16), xs[0:384, 2 * BL:4 * BL]) + thi[i]
    tlo = _dot_nt(jnp.concatenate(klo, axis=1).astype(BF16), xs[0:384, 0:4 * BL])
    st['tm'] = jnp.concatenate([tlo] + thi, axis=0)
    st['ts'] = _dot_nt(xs[384:D, 0:4 * BL], jnp.concatenate(pk[0:4], axis=1).astype(BF16))
    st['z'] = _tree(jnp.add, pk[0:4])
    st['gw'] = jnp.broadcast_to(g_v[...].astype(F32).reshape(1, D), (BL, D)).T
    wait(g3)
    for c in range(4, 9):
        kproj(c)
    tdot(4, 8)
    for c in range(9, 12):
        kproj(c)
    tdot(8, 12)
    wait(g4)
    prep()
    for c in range(12, NB):
        kproj(c)
    tdot(12, NB)
    proj(0, (3, 0))
    kvm = kv_step()
    proj(0, (1, 2))
    attn(0)
    m_step(kvm)
    lin(0)
    proj(1, (3, 0, 1, 2))
    attn(1)
    lin(1)
    final(0)
    proj(2, (3, 0))
    lin(2)
    final(1)
    for c in range(2, NB - 1):
        proj(c, (1, 2))
        attn(c)
        proj(c + 1, (3, 0))
        lin(c + 1)
        if c < NB - 2:
            final(c)
    proj(NB - 1, (1, 2))
    attn(NB - 1)
    final(NB - 2)
    final(NB - 1)
    assert len(cp_o) == NB + 5
    wait(cp_o)


@jax.jit
def pallas_gated_mix__sliding_local_dilated__linear_attn_block__prompt_kernel(
        A_x, A_wqkv, A_wo, B_x, B_wqkv, B_wo, gate_w):
    del B_x
    xt = jnp.swapaxes(A_x, 1, 2).reshape(D, S)
    any_spec = pl.BlockSpec(memory_space=pl.ANY)
    V = pltpu.VMEM
    ot = pl.pallas_call(
        _kernel,
        out_shape=jax.ShapeDtypeStruct((D, S), BF16),
        in_specs=[any_spec] * 6,
        out_specs=any_spec,
        scratch_shapes=[
            V((D, S + BL), BF16),
            V((DP, 3 * D), BF16),
            V((DP, 3 * D), BF16),
            V((D, D), BF16),
            V((D, D), BF16),
            V((D,), BF16),
            V((4, 256, BL), U32),
            V((4, 672, BL), U32),
            V((4, 224, BL), U32),
            V((4, 896, BL), U32),
            V((4, 224, BL), U32),
            V((4, 224, BL), U32),
            V((4, 448, BL), U32),
            V((7, 224, BL), U32),
            V((D, BL), F32),
            V((NB, D, BL), BF16),
            pltpu.SemaphoreType.DMA((5,)),
        ],
        compiler_params=pltpu.CompilerParams(vmem_limit_bytes=64 * 1024 * 1024,
                                             disable_semaphore_checks=True),
    )(xt, A_wqkv, A_wo, B_wqkv, B_wo, gate_w)
    return jnp.swapaxes(ot.reshape(1, D, S), 1, 2)
```

```python
import jax
import jax.numpy as jnp
from jax import lax
import jax.experimental.pallas as pl
import jax.experimental.pallas.tpu as pltpu

S = 2048
D = 448
DP = 512
H = 16
DH = 28
W = 8
DIL = 2
BL = 128
NB = S // BL
DC = 2
JG = 14
NW = 15
F32 = jnp.float32
BF16 = jnp.bfloat16
U32 = jnp.uint32
LOG2E = 1.4426950408889634


def _phi(t):
    return jnp.where(t > 0, t + 1.0, jnp.exp(t)) + 1e-6


def _dot(a, b):
    return jnp.dot(a, b, preferred_element_type=F32)


def _dot_nt(a, b):
    return lax.dot_general(a, b, (((1,), (1,)), ((), ())), preferred_element_type=F32)


def _tree(op, xs):
    xs = list(xs)
    while len(xs) > 1:
        xs = [op(xs[i], xs[i + 1]) if i + 1 < len(xs) else xs[i] for i in range(0, len(xs), 2)]
    return xs[0]


def _bits(x):
    return pltpu.bitcast(x, U32)


def _lanes(ref, r0, n, tiles):
    v = jnp.concatenate([ref[t, r0:r0 + n, :] for t in range(tiles)], axis=1)
    return pltpu.bitcast(v, BF16)


def _interleave_heads(src, src0, dst, dst0):
    for dd in range(DH // 2):
        e = src[:, pl.ds(src0 + dd, 8, stride=DH), :]
        o = src[:, pl.ds(src0 + DH // 2 + dd, 8, stride=DH), :]
        lo = (e & jnp.uint32(0xFFFF)) | (o << 16)
        hi = (e >> 16) | (o & jnp.uint32(0xFFFF0000))
        dst[:, dst0 + 16 * dd:dst0 + 16 * dd + 8, :] = lo
        dst[:, dst0 + 16 * dd + 8:dst0 + 16 * dd + 16, :] = hi


def _heads_f32(src):
    out = []
    for dd in range(DH // 2):
        u = src[:, pl.ds(dd, H, stride=DH // 2), :]
        out.append(pltpu.bitcast(u << 16, F32))
        out.append(pltpu.bitcast(u & jnp.uint32(0xFFFF0000), F32))
    return out


def _kernel(*refs):
    @pl.when(pl.program_id(0) == 0)
    def _():
        _body(*refs)


def _body(x_hbm, wa_hbm, woa_hbm, wb_hbm, wob_hbm, g_hbm, out_hbm,
          xs, wa_v, wb_v, woa_v, wob_v, g_v,
          wkt, tmpa, tmpb, wpt, tmpo, tmpm, tmpv, tt, stack, wcat, ztmp, o_s, sem):
    cpy = pltpu.make_async_copy
    X1, X2, X3 = 2 * BL, 4 * BL, 12 * BL
    g0 = [cpy(wb_hbm.at[:, 640:896], wb_v.at[0:D, 640:896], sem.at[0])]
    g1 = [cpy(x_hbm.at[:, 0:X1], xs.at[:, 0:X1], sem.at[1])]
    g2 = [cpy(wb_hbm.at[:, 384:640], wb_v.at[0:D, 384:640], sem.at[2]),
          cpy(x_hbm.at[:, X1:X2], xs.at[:, X1:X2], sem.at[2]),
          cpy(g_hbm, g_v, sem.at[2])]
    g3 = [cpy(x_hbm.at[:, X2:X3], xs.at[:, X2:X3], sem.at[3])]
    g4 = [cpy(x_hbm.at[:, X3:S], xs.at[:, X3:S], sem.at[4]),
          cpy(wa_hbm, wa_v.at[0:D, :], sem.at[4]),
          cpy(wb_hbm.at[:, 0:384], wb_v.at[0:D, 0:384], sem.at[4]),
          cpy(woa_hbm, woa_v, sem.at[4]),
          cpy(wb_hbm.at[:, 896:1344], wb_v.at[0:D, 896:1344], sem.at[4]),
          cpy(wob_hbm, wob_v, sem.at[4])]
    for cp in g0 + g1 + g2 + g3 + g4:
        cp.start()

    def wait(group):
        for cp in group:
            cp.wait()

    wa_v[D:DP, :] = jnp.zeros((DP - D, 3 * D), BF16)
    wb_v[D:DP, :] = jnp.zeros((DP - D, 3 * D), BF16)

    lane = lax.broadcasted_iota(jnp.int32, (DC, 8, BL), 2)
    lane16 = lax.broadcasted_iota(jnp.int32, (H, BL), 1)

    def zeros_rt(n=BL):
        return _bits(wb_v[D:D + 16, 0:n])

    def xblk(c):
        return xs[:, c * BL:(c + 1) * BL]

    def transpose_cols(src, c0, n, dst, r0):
        t = _bits(src[:, c0:c0 + n].T)
        if dst is wkt:
            t = t | jnp.concatenate([zeros_rt(DP)] * (n // 16), axis=0)
        for ft in range(4):
            dst[ft, r0:r0 + n // 2, :] = t[:, ft * BL:(ft + 1) * BL]

    st = {}
    pk, q_s, qb_s, k_s, kp_s, vp_s, pq_s, g_s, rl_s, ua_s, ub_s = [[None] * NB for _ in range(11)]

    def gate(c, pace):
        p = xblk(c).astype(F32) * st['gw']
        gl = None
        for i0 in range(0, D // 8, 4):
            t = _tree(jnp.add, [p[8 * i:8 * i + 8] for i in range(i0, i0 + 4)])
            t = jnp.where(pace[8 * i0:8 * i0 + 8] > 0, t, 0.0)
            gl = t if gl is None else gl + t
        for sh in (4, 2, 1):
            gl = gl + pltpu.roll(gl, sh, 0)
        g = jax.nn.sigmoid(gl)
        g_s[c] = jnp.concatenate([g, g], axis=0)

    def kproj(c):
        pk[c] = _phi(_dot(_lanes(wkt, 32, 224, 4)[:, 0:D], xblk(c)))
        gate(c, pk[c])
        if c < 8:
            gate(c - 4, pk[c])

    def tdot(c0, c1):
        a = jnp.concatenate(pk[c0:c1], axis=1).astype(BF16)
        st['z'] = _tree(jnp.add, pk[c0:c1]) + st['z']
        st['tm'] = _dot_nt(a, xs[0:384, c0 * BL:c1 * BL]) + st['tm']
        st['ts'] = _dot_nt(xs[384:D, c0 * BL:c1 * BL], a) + st['ts']

    def z_step():
        ztmp[...] = st['z']
        zp = jnp.stack([ztmp[pl.ds(d, H, stride=DH), :] for d in range(DH)])
        st['zb'] = jnp.broadcast_to(jnp.sum(zp, axis=2, keepdims=True), (DH, H, BL))

    def padded_bits(v):
        return jnp.concatenate([_bits(v), jnp.zeros((224, DP - D), U32)], axis=1)

    def stack_t(j):
        wcat[j] = _bits(_lanes(stack, j * 64, 64, 4)[:, 0:D].T)

    def prep():
        for j in range(11):
            transpose_cols(wa_v, j * BL, BL if j < 10 else 64, tmpa, j * 64)
        for p in range(3):
            _interleave_heads(tmpa, p * 224, wpt, p * 224)
        for j in range(3):
            transpose_cols(wb_v, j * BL, BL, tmpb, j * 64)
        tmpb[:, 192:224, :] = wkt[:, 0:32, :]
        _interleave_heads(tmpb, 0, wpt, 3 * 224)
        u = padded_bits(woa_v[...])
        for nt in range(4):
            tmpo[nt] = u[:, nt * BL:(nt + 1) * BL]
        _interleave_heads(tmpo, 0, stack, 224)
        for j in range(4, 7):
            stack_t(j)

    def m_step(pace):
        zero = zeros_rt()
        tm = _bits(st['tm'])

        def anchor(i):
            return tm[8 * (i % 56):8 * (i % 56) + 8, (i // 56) * BL:(i // 56 + 1) * BL] & zero

        for j in range(4):
            transpose_cols(wb_v, 896 + j * BL, BL if j < 3 else 64, tmpv, j * 64)
        wv = _heads_f32(tmpv)
        u = padded_bits(wob_v[...])
        for r in range(DH):
            a = anchor(3 * r)
            for nt in range(4):
                tmpm[nt, 8 * r:8 * r + 8, :] = u[8 * r:8 * r + 8, nt * BL:(nt + 1) * BL] | a
        wo = _heads_f32(tmpm)
        for t in range(3):
            tt[t] = st['tm'][:, t * BL:(t + 1) * BL]
        tt[3] = jnp.concatenate([st['ts'], jnp.zeros((DP - D, D), F32)], axis=0).T
        pins = []
        for j in range(DH):
            for tab, i in ((wo, 100 + (j * 68) // DH), (wv, 30 + ((2 * j + 1) * 138) // (2 * DH))):
                b = _bits(tab[j])
                b = _tree(jnp.bitwise_or, [b[t, 8 * h:8 * h + 8] for t in range(4) for h in range(2)])
                pins.append(pltpu.roll(b & anchor(i), 1, 1))
        zero = zero | _tree(jnp.bitwise_or, pins)
        zero = jnp.concatenate([zero, zero], axis=0)
        p0, p1, first = 100, 1670, 56
        ngrp = (DH - 1) * (DH // JG)
        hist, mp, pinned = [], [], 0
        for d in range(DH):
            td = _bits(tt[:, pl.ds(d, H, stride=DH), :])
            m = None
            for j0 in range(0, DH, JG):
                if d == 0:
                    pi = p0 + (j0 * first) // DH
                else:
                    pi = p0 + first + ((len(hist) - DH // JG) * (p1 - p0 - first)) // ngrp
                zg = zero & _bits(pace[pi // 2])
                if pi >= 112 * pinned + 96:
                    zg = zg & _bits(rl_s[pinned])
                    pinned += 1
                tie = (_bits(hist[-2]) & zg[None]) if len(hist) >= 2 else zg[None]
                tg = pltpu.bitcast(td | tie, F32)
                for j in range(j0, j0 + JG):
                    s = (tg[0] * wv[j][0] + tg[1] * wv[j][1]) + (tg[2] * wv[j][2] + tg[3] * wv[j][3])
                    p = jnp.sum(s, axis=1, keepdims=True)[None] * wo[j]
                    m = p if m is None else m + p
                hist.append(m)
            mp.append(_bits(m.astype(BF16)))
        last = mp[-1][0] & zero[0:8]
        for d in range(DH):
            stack[:, 8 * d:8 * d + 8, :] = (mp[d] | last[None]) if d % 8 == 0 else mp[d]
        for j in range(4):
            stack_t(j)

    def proj(c, parts):
        x = xblk(c)
        for p in parts:
            r = _dot(_lanes(wpt, p * 224, 224, 4)[:, 0:D], x)
            if p == 0:
                q_s[c] = r.reshape(DH, H, BL)
            elif p == 1:
                k_s[c] = r.reshape(DH, H, BL)
                kp_s[c] = _bits(r.astype(BF16)).reshape(DH, 8, BL)
            elif p == 2:
                vp_s[c] = _bits(r.astype(BF16)).reshape(DH, 8, BL)
            else:
                qb_s[c] = r.reshape(DH, H, BL)
                pq_s[c] = _phi(r).reshape(DH, H, BL)

    def shifted(vals, c, d0, w, ln):
        sh = vals[c][d0:d0 + DC]
        if w > 0:
            if c > 0:
                sh = jnp.where(ln >= BL - DIL * w, vals[c - 1][d0:d0 + DC], sh)
            sh = pltpu.roll(sh, DIL * w, 2)
        return pltpu.bitcast(sh, BF16).astype(F32)

    def attn(c):
        logit = [None] * W
        for d0 in range(0, DH, DC):
            q = q_s[c][d0:d0 + DC]
            for w in range(W):
                k = k_s[c][d0:d0 + DC] if w == 0 else shifted(kp_s, c, d0, w, lane)
                p = jnp.sum(q * k, axis=0)
                logit[w] = p if logit[w] is None else logit[w] + p
        if c == 0:
            logit = [jnp.where(lane16 >= DIL * w, l, -1e9 * DH ** 0.5) for w, l in enumerate(logit)]
        m = _tree(jnp.maximum, logit)
        e = [jnp.exp2((l - m) * (DH ** -0.5 * LOG2E)) for l in logit]
        r = g_s[c] / _tree(jnp.add, e)
        mb = pltpu.bitcast(m, jnp.int32)
        ln = lane[0] | (mb[0:8] & mb[8:16] & pltpu.bitcast(zeros_rt(), jnp.int32))
        ln = jnp.broadcast_to(ln[None], lane.shape)
        us = []
        for d0 in range(0, DH, DC):
            o = None
            for w in range(W):
                p = e[w][None] * shifted(vp_s, c, d0, w, ln)
                o = p if o is None else o + p
            us.append(o * r[None])
        ua_s[c] = jnp.concatenate(us, axis=0)

    def lin(c):
        pq = pq_s[c]
        den = jnp.sum(pq * st['zb'], axis=0) + 1e-6
        rl_s[c] = (1.0 - g_s[c]) / den
        ub_s[c] = pq * rl_s[c][None]

    cp_o = []

    def final(c):
        u = jnp.concatenate([ub_s[c], ua_s[c]], axis=0).reshape(2 * D, BL)
        u0, u1 = u[0:384].astype(BF16), u[384:].astype(BF16)
        wl = [_lanes(wcat, 56 * i, 56, 7) for i in range(4)]
        o = [None] * 4
        for i0 in (0, 2):
            pb = [_dot(wl[i][:, 0:384], u0) for i in (i0, i0 + 1)]
            for i in (i0, i0 + 1):
                o[i] = _dot(wl[i][:, 384:], u1) + pb[i - i0]
        o = jnp.concatenate(o, axis=0)
        cuts = (0, 112, 224, 336, 400, 432, D) if c == NB - 1 else (0, D)
        for r0, r1 in zip(cuts[:-1], cuts[1:]):
            o_s[c, r0:r1, :] = o[r0:r1].astype(BF16)
            cp = cpy(o_s.at[c, r0:r1, :], out_hbm.at[r0:r1, c * BL:(c + 1) * BL], sem.at[0])
            cp.start()
            cp_o.append(cp)

    wait(g0)
    for j in (2, 3):
        transpose_cols(wb_v, 384 + j * BL, BL, wkt, j * 64)
    wait(g1)
    whi = _lanes(wkt, 128, 128, 4)[:, 0:D]
    khi = [_phi(_dot(whi, xblk(c))) for c in range(2)]
    thi = [None, None]
    for c in range(2):
        for i in range(2):
            t = _dot_nt(khi[c][i * BL:(i + 1) * BL].astype(BF16), xs[0:384, c * BL:(c + 1) * BL])
            thi[i] = t if thi[i] is None else t + thi[i]
    wait(g2)
    khi += [_phi(_dot(whi, xblk(c))) for c in range(2, 4)]
    for j in (0, 1):
        transpose_cols(wb_v, 384 + j * BL, BL, wkt, j * 64)
    wlo = _lanes(wkt, 32, 96, 4)[:, 0:D]
    klo = [_phi(_dot(wlo, xblk(c))) for c in range(4)]
    for c in range(4):
        pk[c] = jnp.concatenate([klo[c], khi[c]], axis=0)
    for i in range(2):
        a = jnp.concatenate([khi[2][i * BL:(i + 1) * BL], khi[3][i * BL:(i + 1) * BL]], axis=1)
        thi[i] = _dot_nt(a.astype(BF16), xs[0:384, 2 * BL:4 * BL]) + thi[i]
    tlo = _dot_nt(jnp.concatenate(klo, axis=1).astype(BF16), xs[0:384, 0:4 * BL])
    st['tm'] = jnp.concatenate([tlo] + thi, axis=0)
    st['ts'] = _dot_nt(xs[384:D, 0:4 * BL], jnp.concatenate(pk[0:4], axis=1).astype(BF16))
    st['z'] = _tree(jnp.add, pk[0:4])
    st['gw'] = jnp.broadcast_to(g_v[...].astype(F32).reshape(1, D), (BL, D)).T
    wait(g3)
    for c in range(4, 9):
        kproj(c)
    tdot(4, 8)
    for c in range(9, 12):
        kproj(c)
    tdot(8, 12)
    wait(g4)
    prep()
    for c in range(12, NB):
        kproj(c)
    tdot(12, NB)
    z_step()
    pace = []
    for c in range(NW):
        proj(c, (3, 0))
        lin(c)
        pace += [qb_s[c][i] for i in range(DH)] + [q_s[c][i] for i in range(DH)]
    m_step(pace)
    rest = [(c, p) for c in range(NW, NB) for p in (3, 0)]
    proj(0, (1,))
    proj(rest[0][0], (rest[0][1],))
    proj(0, (2,))
    attn(0)
    for c, p in rest[1:]:
        proj(c, (p,))
    for c in range(NW, NB):
        lin(c)
    for c in range(1, NB - 1):
        proj(c, (2, 1))
        attn(c)
        if c < NB - 2:
            final(c - 1)
    proj(NB - 1, (1, 2))
    attn(NB - 1)
    for c in range(NB - 3, NB):
        final(c)
    assert len(cp_o) == NB + 5
    wait(cp_o)


@jax.jit
def pallas_gated_mix__sliding_local_dilated__linear_attn_block__prompt_kernel(
        A_x, A_wqkv, A_wo, B_x, B_wqkv, B_wo, gate_w):
    del B_x
    xt = jnp.swapaxes(A_x, 1, 2).reshape(D, S)
    any_spec = pl.BlockSpec(memory_space=pl.ANY)
    V = pltpu.VMEM
    ot = pl.pallas_call(
        _kernel,
        out_shape=jax.ShapeDtypeStruct((D, S), BF16),
        grid=(2,),
        in_specs=[any_spec] * 6,
        out_specs=any_spec,
        scratch_shapes=[
            V((D, S + BL), BF16),
            V((DP, 3 * D), BF16),
            V((DP, 3 * D), BF16),
            V((D, D), BF16),
            V((D, D), BF16),
            V((D,), BF16),
            V((4, 256, BL), U32),
            V((4, 672, BL), U32),
            V((4, 224, BL), U32),
            V((4, 896, BL), U32),
            V((4, 224, BL), U32),
            V((4, 224, BL), U32),
            V((4, 224, BL), U32),
            V((4, D, BL), F32),
            V((4, 448, BL), U32),
            V((7, 224, BL), U32),
            V((D, BL), F32),
            V((NB, D, BL), BF16),
            pltpu.SemaphoreType.DMA((5,)),
        ],
        compiler_params=pltpu.CompilerParams(dimension_semantics=("arbitrary",),
                                             vmem_limit_bytes=64 * 1024 * 1024,
                                             disable_semaphore_checks=True),
    )(xt, A_wqkv, A_wo, B_wqkv, B_wo, gate_w)
    return jnp.swapaxes(ot.reshape(1, D, S), 1, 2)
```

```python
import jax
import jax.numpy as jnp
from jax import lax
import jax.experimental.pallas as pl
import jax.experimental.pallas.tpu as pltpu

S = 2048
D = 448
DP = 512
H = 16
DH = 28
W = 8
DIL = 2
BL = 128
NB = S // BL
JG = 14
NW = 15
F32 = jnp.float32
BF16 = jnp.bfloat16
U32 = jnp.uint32
LOG2E = 1.4426950408889634


def _phi(t):
    return jnp.where(t > 0, t + 1.0, jnp.exp(t)) + 1e-6


def _dot(a, b):
    return jnp.dot(a, b, preferred_element_type=F32)


def _dot_nt(a, b):
    return lax.dot_general(a, b, (((1,), (1,)), ((), ())), preferred_element_type=F32)


def _tree(op, xs):
    xs = list(xs)
    while len(xs) > 1:
        xs = [op(xs[i], xs[i + 1]) if i + 1 < len(xs) else xs[i] for i in range(0, len(xs), 2)]
    return xs[0]


def _bits(x):
    return pltpu.bitcast(x, U32)


def _lanes(ref, r0, n, tiles):
    v = jnp.concatenate([ref[t, r0:r0 + n, :] for t in range(tiles)], axis=1)
    return pltpu.bitcast(v, BF16)


def _interleave_heads(src, src0, dst, dst0):
    for dd in range(DH // 2):
        e = src[:, pl.ds(src0 + dd, 8, stride=DH), :]
        o = src[:, pl.ds(src0 + DH // 2 + dd, 8, stride=DH), :]
        lo = (e & jnp.uint32(0xFFFF)) | (o << 16)
        hi = (e >> 16) | (o & jnp.uint32(0xFFFF0000))
        dst[:, dst0 + 16 * dd:dst0 + 16 * dd + 8, :] = lo
        dst[:, dst0 + 16 * dd + 8:dst0 + 16 * dd + 16, :] = hi


def _heads_f32(src):
    out = []
    for dd in range(DH // 2):
        u = src[:, pl.ds(dd, H, stride=DH // 2), :]
        out.append(pltpu.bitcast(u << 16, F32))
        out.append(pltpu.bitcast(u & jnp.uint32(0xFFFF0000), F32))
    return out


def _kernel(*refs):
    @pl.when(pl.program_id(0) == 0)
    def _():
        _body(*refs)


def _body(x_hbm, wa_hbm, woa_hbm, wb_hbm, wob_hbm, g_hbm, out_hbm,
          xs, wa_v, wb_v, woa_v, wob_v, g_v,
          wkt, tmpa, tmpb, wpt, tmpo, tmpm, tmpv, tt, stack, wcat, ztmp, o_s, sem):
    cpy = pltpu.make_async_copy
    X1, X2, X3 = 2 * BL, 4 * BL, 12 * BL
    g0 = [cpy(wb_hbm.at[:, 640:896], wb_v.at[0:D, 640:896], sem.at[0])]
    g1 = [cpy(x_hbm.at[:, 0:X1], xs.at[:, 0:X1], sem.at[1])]
    g2 = [cpy(wb_hbm.at[:, 384:640], wb_v.at[0:D, 384:640], sem.at[2]),
          cpy(x_hbm.at[:, X1:X2], xs.at[:, X1:X2], sem.at[2]),
          cpy(g_hbm, g_v, sem.at[2])]
    g3 = [cpy(x_hbm.at[:, X2:X3], xs.at[:, X2:X3], sem.at[3])]
    g4 = [cpy(x_hbm.at[:, X3:S], xs.at[:, X3:S], sem.at[4]),
          cpy(wa_hbm, wa_v.at[0:D, :], sem.at[4]),
          cpy(wb_hbm.at[:, 0:384], wb_v.at[0:D, 0:384], sem.at[4]),
          cpy(woa_hbm, woa_v, sem.at[4]),
          cpy(wb_hbm.at[:, 896:1344], wb_v.at[0:D, 896:1344], sem.at[4]),
          cpy(wob_hbm, wob_v, sem.at[4])]
    for cp in g0 + g1 + g2 + g3 + g4:
        cp.start()

    def wait(group):
        for cp in group:
            cp.wait()

    wa_v[D:DP, :] = jnp.zeros((DP - D, 3 * D), BF16)
    wb_v[D:DP, :] = jnp.zeros((DP - D, 3 * D), BF16)

    lane = lax.broadcasted_iota(jnp.int32, (8, BL), 1)
    lane16 = lax.broadcasted_iota(jnp.int32, (H, BL), 1)

    def zeros_rt(n=BL):
        return _bits(wb_v[D:D + 16, 0:n])

    def xblk(c):
        return xs[:, c * BL:(c + 1) * BL]

    def transpose_cols(src, c0, n, dst, r0):
        t = _bits(src[:, c0:c0 + n].T)
        if dst is wkt:
            t = t | jnp.concatenate([zeros_rt(DP)] * (n // 16), axis=0)
        for ft in range(4):
            dst[ft, r0:r0 + n // 2, :] = t[:, ft * BL:(ft + 1) * BL]

    st = {}
    pk, q_s, qb_s, k_s, kp_s, vp_s, pq_s, g_s, rl_s, ua_s, ub_s = [[None] * NB for _ in range(11)]

    def gate(c, pace):
        p = (xblk(c).astype(F32) * st['gw']).reshape(D // 32, 4, 8, BL)
        t = (p[:, 0] + p[:, 1]) + (p[:, 2] + p[:, 3])
        gl = jnp.sum(jnp.where(pace.reshape(D // 32, 4, 8, BL)[:, 0] > 0, t, 0.0), axis=0)
        for sh in (4, 2, 1):
            gl = gl + pltpu.roll(gl, sh, 0)
        g = jax.nn.sigmoid(gl)
        g_s[c] = jnp.concatenate([g, g], axis=0)

    def kproj(c):
        pk[c] = _phi(_dot(_lanes(wkt, 32, 224, 4)[:, 0:D], xblk(c)))
        gate(c, pk[c])
        if c < 8:
            gate(c - 4, pk[c])

    def tdot(c0, c1):
        a = jnp.concatenate(pk[c0:c1], axis=1).astype(BF16)
        st['z'] = _tree(jnp.add, pk[c0:c1]) + st['z']
        st['tm'] = _dot_nt(a, xs[0:384, c0 * BL:c1 * BL]) + st['tm']
        st['ts'] = _dot_nt(xs[384:D, c0 * BL:c1 * BL], a) + st['ts']

    def z_step():
        ztmp[...] = st['z']
        zp = jnp.stack([ztmp[pl.ds(d, H, stride=DH), :] for d in range(DH)])
        st['zb'] = jnp.broadcast_to(jnp.sum(zp, axis=2, keepdims=True), (DH, H, BL))

    def padded_bits(v):
        return jnp.concatenate([_bits(v), jnp.zeros((224, DP - D), U32)], axis=1)

    def stack_t(j):
        wcat[j] = _bits(_lanes(stack, j * 64, 64, 4)[:, 0:D].T)

    def prep():
        for j in range(11):
            transpose_cols(wa_v, j * BL, BL if j < 10 else 64, tmpa, j * 64)
        for p in range(3):
            _interleave_heads(tmpa, p * 224, wpt, p * 224)
        for j in range(3):
            transpose_cols(wb_v, j * BL, BL, tmpb, j * 64)
        tmpb[:, 192:224, :] = wkt[:, 0:32, :]
        _interleave_heads(tmpb, 0, wpt, 3 * 224)
        u = padded_bits(woa_v[...])
        for nt in range(4):
            tmpo[nt] = u[:, nt * BL:(nt + 1) * BL]
        _interleave_heads(tmpo, 0, stack, 224)
        for j in range(4, 7):
            stack_t(j)

    def m_step(pace):
        zero = zeros_rt()
        tm = _bits(st['tm'])

        def anchor(i):
            return tm[8 * (i % 56):8 * (i % 56) + 8, (i // 56) * BL:(i // 56 + 1) * BL] & zero

        for j in range(4):
            transpose_cols(wb_v, 896 + j * BL, BL if j < 3 else 64, tmpv, j * 64)
        wv = _heads_f32(tmpv)
        u = padded_bits(wob_v[...])
        for r in range(DH):
            a = anchor(3 * r)
            for nt in range(4):
                tmpm[nt, 8 * r:8 * r + 8, :] = u[8 * r:8 * r + 8, nt * BL:(nt + 1) * BL] | a
        wo = _heads_f32(tmpm)
        for t in range(3):
            tt[t] = st['tm'][:, t * BL:(t + 1) * BL]
        tt[3] = jnp.concatenate([st['ts'], jnp.zeros((DP - D, D), F32)], axis=0).T
        pins = []
        for j in range(DH):
            for tab, i in ((wo, 100 + (j * 68) // DH), (wv, 30 + ((2 * j + 1) * 138) // (2 * DH))):
                b = _bits(tab[j])
                b = _tree(jnp.bitwise_or, [b[t, 8 * h:8 * h + 8] for t in range(4) for h in range(2)])
                pins.append(pltpu.roll(b & anchor(i), 1, 1))
        zero = zero | _tree(jnp.bitwise_or, pins)
        zero = jnp.concatenate([zero, zero], axis=0)
        p0, p1, first = 90, 1670, 56
        ngrp = (DH - 1) * (DH // JG)
        hist, mp, pinned = [], [], 0
        wvg = [jnp.stack(wv[j0:j0 + JG]) for j0 in range(0, DH, JG)]
        wog = [jnp.stack(wo[j0:j0 + JG]) for j0 in range(0, DH, JG)]
        for d in range(DH):
            td = _bits(tt[:, pl.ds(d, H, stride=DH), :])
            m = None
            for j0 in range(0, DH, JG):
                if d == 0:
                    pi = p0 + (j0 * first) // DH
                else:
                    pi = p0 + first + ((len(hist) - DH // JG) * (p1 - p0 - first)) // ngrp
                pv, pr_ = pace[pi // 2]
                zg = zero & _bits(pv[pr_])
                if pi >= 112 * pinned + 96:
                    zg = zg & _bits(rl_s[pinned])
                    pinned += 1
                tie = (_bits(hist[-2]) & zg[None]) if len(hist) >= 2 else zg[None]
                tg = pltpu.bitcast(td | tie, F32)
                pr = tg[None] * wvg[j0 // JG]
                kv = jnp.sum((pr[:, 0] + pr[:, 1]) + (pr[:, 2] + pr[:, 3]), axis=2, keepdims=True)
                p = kv[:, None] * wog[j0 // JG]
                if m is not None:
                    p = jnp.concatenate([m[None], p], axis=0)
                m = jnp.sum(p, axis=0)
                hist.append(m)
            mp.append(_bits(m.astype(BF16)))
        last = mp[-1][0] & zero[0:8]
        for d in range(DH):
            stack[:, 8 * d:8 * d + 8, :] = (mp[d] | last[None]) if d % 8 == 0 else mp[d]
        for j in range(4):
            stack_t(j)

    def proj(c, parts):
        x = xblk(c)
        for p in parts:
            r = _dot(_lanes(wpt, p * 224, 224, 4)[:, 0:D], x)
            if p == 0:
                q_s[c] = r.reshape(DH, H, BL)
            elif p == 1:
                k_s[c] = r.reshape(DH, H, BL)
                kp_s[c] = _bits(r.astype(BF16)).reshape(DH, 8, BL)
            elif p == 2:
                vp_s[c] = _bits(r.astype(BF16)).reshape(DH, 8, BL)
            else:
                qb_s[c] = r.reshape(DH, H, BL)
                pq_s[c] = _phi(r).reshape(DH, H, BL)

    def masks(ln):
        return [None] + [jnp.broadcast_to((ln >= BL - DIL * w)[None], (DH, 8, BL)) for w in range(1, W)]

    def shifted(vals, c, w, msk):
        cur = vals[c]
        if w > 0:
            if c > 0:
                cur = lax.select(msk[w], vals[c - 1], cur)
            cur = pltpu.roll(cur, DIL * w, 2)
        return pltpu.bitcast(cur, BF16).astype(F32)

    def attn(c):
        logit = []
        for w in range(W):
            k = k_s[c] if w == 0 else shifted(kp_s, c, w, st['msk'])
            logit.append(jnp.sum(q_s[c] * k, axis=0))
        if c == 0:
            logit = [jnp.where(lane16 >= DIL * w, l, -1e9 * DH ** 0.5) for w, l in enumerate(logit)]
        m = _tree(jnp.maximum, logit)
        e = [jnp.exp2((l - m) * (DH ** -0.5 * LOG2E)) for l in logit]
        r = g_s[c] / _tree(jnp.add, e)
        mb = pltpu.bitcast(m, jnp.int32)
        msk = masks(lane | (mb[0:8] & mb[8:16] & pltpu.bitcast(zeros_rt(), jnp.int32)))
        o = None
        for w in range(W):
            p = e[w][None] * shifted(vp_s, c, w, msk)
            o = p if o is None else o + p
        ua_s[c] = o * r[None]

    def lin(c):
        pq = pq_s[c]
        den = jnp.sum(pq * st['zb'], axis=0) + 1e-6
        rl_s[c] = (1.0 - g_s[c]) / den
        ub_s[c] = pq * rl_s[c][None]

    cp_o = []

    def final(c):
        u = jnp.concatenate([ub_s[c], ua_s[c]], axis=0).reshape(2 * D, BL)
        u0, u1 = u[0:384].astype(BF16), u[384:].astype(BF16)
        wl = [_lanes(wcat, 56 * i, 56, 7) for i in range(4)]
        o = [None] * 4
        for i0 in (0, 2):
            pb = [_dot(wl[i][:, 0:384], u0) for i in (i0, i0 + 1)]
            for i in (i0, i0 + 1):
                o[i] = _dot(wl[i][:, 384:], u1) + pb[i - i0]
        o = jnp.concatenate(o, axis=0)
        cuts = (0, 112, 224, 336, 400, 432, D) if c == NB - 1 else (0, D)
        for r0, r1 in zip(cuts[:-1], cuts[1:]):
            o_s[c, r0:r1, :] = o[r0:r1].astype(BF16)
            cp = cpy(o_s.at[c, r0:r1, :], out_hbm.at[r0:r1, c * BL:(c + 1) * BL], sem.at[0])
            cp.start()
            cp_o.append(cp)

    wait(g0)
    for j in (2, 3):
        transpose_cols(wb_v, 384 + j * BL, BL, wkt, j * 64)
    wait(g1)
    whi = _lanes(wkt, 128, 128, 4)[:, 0:D]
    khi = [_phi(_dot(whi, xblk(c))) for c in range(2)]
    thi = [None, None]
    for c in range(2):
        for i in range(2):
            t = _dot_nt(khi[c][i * BL:(i + 1) * BL].astype(BF16), xs[0:384, c * BL:(c + 1) * BL])
            thi[i] = t if thi[i] is None else t + thi[i]
    wait(g2)
    khi += [_phi(_dot(whi, xblk(c))) for c in range(2, 4)]
    for j in (0, 1):
        transpose_cols(wb_v, 384 + j * BL, BL, wkt, j * 64)
    wlo = _lanes(wkt, 32, 96, 4)[:, 0:D]
    klo = [_phi(_dot(wlo, xblk(c))) for c in range(4)]
    for c in range(4):
        pk[c] = jnp.concatenate([klo[c], khi[c]], axis=0)
    for i in range(2):
        a = jnp.concatenate([khi[2][i * BL:(i + 1) * BL], khi[3][i * BL:(i + 1) * BL]], axis=1)
        thi[i] = _dot_nt(a.astype(BF16), xs[0:384, 2 * BL:4 * BL]) + thi[i]
    tlo = _dot_nt(jnp.concatenate(klo, axis=1).astype(BF16), xs[0:384, 0:4 * BL])
    st['tm'] = jnp.concatenate([tlo] + thi, axis=0)
    st['ts'] = _dot_nt(xs[384:D, 0:4 * BL], jnp.concatenate(pk[0:4], axis=1).astype(BF16))
    st['z'] = _tree(jnp.add, pk[0:4])
    st['gw'] = jnp.broadcast_to(g_v[...].astype(F32).reshape(1, D), (BL, D)).T
    wait(g3)
    for c in range(4, 9):
        kproj(c)
    tdot(4, 8)
    for c in range(9, 12):
        kproj(c)
    tdot(8, 12)
    wait(g4)
    prep()
    for c in range(12, NB):
        kproj(c)
    tdot(12, NB)
    z_step()
    pace = []
    for c in range(NW):
        proj(c, (3, 0))
        lin(c)
        pace += [(qb_s[c], i) for i in range(DH)] + [(q_s[c], i) for i in range(DH)]
    m_step(pace)
    st['msk'] = masks(lane)
    rest = [(c, p) for c in range(NW, NB) for p in (3, 0)]
    proj(0, (1,))
    proj(rest[0][0], (rest[0][1],))
    proj(0, (2,))
    attn(0)
    for c, p in rest[1:]:
        proj(c, (p,))
    for c in range(NW, NB):
        lin(c)
    for c in range(1, NB - 1):
        proj(c, (2, 1))
        attn(c)
        if c < NB - 2:
            final(c - 1)
    proj(NB - 1, (1, 2))
    attn(NB - 1)
    for c in range(NB - 3, NB):
        final(c)
    assert len(cp_o) == NB + 5
    wait(cp_o)


@jax.jit
def pallas_gated_mix__sliding_local_dilated__linear_attn_block__prompt_kernel(
        A_x, A_wqkv, A_wo, B_x, B_wqkv, B_wo, gate_w):
    del B_x
    xt = jnp.swapaxes(A_x, 1, 2).reshape(D, S)
    any_spec = pl.BlockSpec(memory_space=pl.ANY)
    V = pltpu.VMEM
    ot = pl.pallas_call(
        _kernel,
        out_shape=jax.ShapeDtypeStruct((D, S), BF16),
        grid=(2,),
        in_specs=[any_spec] * 6,
        out_specs=any_spec,
        scratch_shapes=[
            V((D, S + BL), BF16),
            V((DP, 3 * D), BF16),
            V((DP, 3 * D), BF16),
            V((D, D), BF16),
            V((D, D), BF16),
            V((D,), BF16),
            V((4, 256, BL), U32),
            V((4, 672, BL), U32),
            V((4, 224, BL), U32),
            V((4, 896, BL), U32),
            V((4, 224, BL), U32),
            V((4, 224, BL), U32),
            V((4, 224, BL), U32),
            V((4, D, BL), F32),
            V((4, 448, BL), U32),
            V((7, 224, BL), U32),
            V((D, BL), F32),
            V((NB, D, BL), BF16),
            pltpu.SemaphoreType.DMA((5,)),
        ],
        compiler_params=pltpu.CompilerParams(dimension_semantics=("arbitrary",),
                                             vmem_limit_bytes=64 * 1024 * 1024,
                                             disable_semaphore_checks=True),
    )(xt, A_wqkv, A_wo, B_wqkv, B_wo, gate_w)
    return jnp.swapaxes(ot.reshape(1, D, S), 1, 2)
```

```python
import jax
import jax.numpy as jnp
from jax import lax
import jax.experimental.pallas as pl
import jax.experimental.pallas.tpu as pltpu

S = 2048
D = 448
DP = 512
H = 16
DH = 28
W = 8
DIL = 2
BL = 128
NB = S // BL
JG = 14
NW = 15
F32 = jnp.float32
BF16 = jnp.bfloat16
U32 = jnp.uint32
LOG2E = 1.4426950408889634


def _phi(t):
    return jnp.where(t > 0, t + 1.0, jnp.exp(t)) + 1e-6


def _dot(a, b):
    return jnp.dot(a, b, preferred_element_type=F32)


def _dot_nt(a, b):
    return lax.dot_general(a, b, (((1,), (1,)), ((), ())), preferred_element_type=F32)


def _tree(op, xs):
    xs = list(xs)
    while len(xs) > 1:
        xs = [op(xs[i], xs[i + 1]) if i + 1 < len(xs) else xs[i] for i in range(0, len(xs), 2)]
    return xs[0]


def _bits(x):
    return pltpu.bitcast(x, U32)


def _lanes(ref, r0, n, tiles):
    v = jnp.concatenate([ref[t, r0:r0 + n, :] for t in range(tiles)], axis=1)
    return pltpu.bitcast(v, BF16)


def _interleave_heads(src, src0, dst, dst0):
    for dd in range(DH // 2):
        e = src[:, pl.ds(src0 + dd, 8, stride=DH), :]
        o = src[:, pl.ds(src0 + DH // 2 + dd, 8, stride=DH), :]
        lo = (e & jnp.uint32(0xFFFF)) | (o << 16)
        hi = (e >> 16) | (o & jnp.uint32(0xFFFF0000))
        dst[:, dst0 + 16 * dd:dst0 + 16 * dd + 8, :] = lo
        dst[:, dst0 + 16 * dd + 8:dst0 + 16 * dd + 16, :] = hi


def _heads_f32(src):
    out = []
    for dd in range(DH // 2):
        u = src[:, pl.ds(dd, H, stride=DH // 2), :]
        out.append(pltpu.bitcast(u << 16, F32))
        out.append(pltpu.bitcast(u & jnp.uint32(0xFFFF0000), F32))
    return out


def _kernel(*refs):
    @pl.when(pl.program_id(0) == 0)
    def _():
        _body(*refs)


def _body(x_hbm, wa_hbm, woa_hbm, wb_hbm, wob_hbm, g_hbm, out_hbm,
          xs, wa_v, wb_v, woa_v, wob_v, g_v,
          wkt, tmpa, tmpb, wpt, tmpo, tmpm, tmpv, tt, stack, wcat, ztmp, o_s, sem):
    cpy = pltpu.make_async_copy
    X1, X2, X3 = 2 * BL, 4 * BL, 12 * BL
    g0 = [cpy(wb_hbm.at[:, 640:896], wb_v.at[0:D, 640:896], sem.at[0])]
    g1 = [cpy(x_hbm.at[:, 0:X1], xs.at[:, 0:X1], sem.at[1])]
    g2 = [cpy(wb_hbm.at[:, 384:640], wb_v.at[0:D, 384:640], sem.at[2]),
          cpy(x_hbm.at[:, X1:X2], xs.at[:, X1:X2], sem.at[2]),
          cpy(g_hbm, g_v, sem.at[2])]
    g3 = [cpy(x_hbm.at[:, X2:X3], xs.at[:, X2:X3], sem.at[3])]
    g4 = [cpy(x_hbm.at[:, X3:S], xs.at[:, X3:S], sem.at[4]),
          cpy(wa_hbm, wa_v.at[0:D, :], sem.at[4]),
          cpy(wb_hbm.at[:, 0:384], wb_v.at[0:D, 0:384], sem.at[4]),
          cpy(woa_hbm, woa_v, sem.at[4]),
          cpy(wb_hbm.at[:, 896:1344], wb_v.at[0:D, 896:1344], sem.at[4]),
          cpy(wob_hbm, wob_v, sem.at[4])]
    for cp in g0 + g1 + g2 + g3 + g4:
        cp.start()

    def wait(group):
        for cp in group:
            cp.wait()

    wa_v[D:DP, :] = jnp.zeros((DP - D, 3 * D), BF16)
    wb_v[D:DP, :] = jnp.zeros((DP - D, 3 * D), BF16)

    lane = lax.broadcasted_iota(jnp.int32, (8, BL), 1)
    lane16 = lax.broadcasted_iota(jnp.int32, (H, BL), 1)

    def zeros_rt(n=BL):
        return _bits(wb_v[D:D + 16, 0:n])

    def xblk(c):
        return xs[:, c * BL:(c + 1) * BL]

    def transpose_cols(src, c0, n, dst, r0):
        t = _bits(src[:, c0:c0 + n].T)
        if dst is wkt:
            t = t | jnp.concatenate([zeros_rt(DP)] * (n // 16), axis=0)
        for ft in range(4):
            dst[ft, r0:r0 + n // 2, :] = t[:, ft * BL:(ft + 1) * BL]

    st = {}
    pk, q_s, qb_s, k_s, kp_s, vp_s, pq_s, g_s, rl_s, ua_s, ub_s = [[None] * NB for _ in range(11)]

    def gate(c, pace):
        p = (xblk(c).astype(F32) * st['gw']).reshape(D // 32, 4, 8, BL)
        t = (p[:, 0] + p[:, 1]) + (p[:, 2] + p[:, 3])
        gl = jnp.sum(jnp.where(pace.reshape(D // 32, 4, 8, BL)[:, 0] > 0, t, 0.0), axis=0)
        for sh in (4, 2, 1):
            gl = gl + pltpu.roll(gl, sh, 0)
        g = jax.nn.sigmoid(gl)
        g_s[c] = jnp.concatenate([g, g], axis=0)

    def kproj(c):
        pk[c] = _phi(_dot(_lanes(wkt, 32, 224, 4)[:, 0:D], xblk(c)))
        gate(c, pk[c])
        if c < 8:
            gate(c - 4, pk[c])

    def tdot(c0, c1):
        a = jnp.concatenate(pk[c0:c1], axis=1).astype(BF16)
        st['z'] = _tree(jnp.add, pk[c0:c1]) + st['z']
        st['tm'] = _dot_nt(a, xs[0:384, c0 * BL:c1 * BL]) + st['tm']
        st['ts'] = _dot_nt(xs[384:D, c0 * BL:c1 * BL], a) + st['ts']

    def z_step():
        ztmp[0:D, :] = st['z']
        zp = jnp.stack([ztmp[pl.ds(d, H, stride=DH), :] for d in range(DH)])
        st['zb'] = jnp.broadcast_to(jnp.sum(zp, axis=2, keepdims=True), (DH, H, BL))

    def padded_bits(v):
        return jnp.concatenate([_bits(v), jnp.zeros((224, DP - D), U32)], axis=1)

    def stack_t(j, tie=None):
        if tie is not None:
            stack[:, j * 64:j * 64 + 8, :] = stack[:, j * 64:j * 64 + 8, :] | tie[None]
        wcat[j] = _bits(_lanes(stack, j * 64, 64, 4)[:, 0:D].T)

    def prep():
        for j in range(3):
            transpose_cols(wb_v, j * BL, BL, tmpb, j * 64)
        tmpb[:, 192:224, :] = wkt[:, 0:32, :]
        _interleave_heads(tmpb, 0, wpt, 3 * 224)
        for j in range(11):
            transpose_cols(wa_v, j * BL, BL if j < 10 else 64, tmpa, j * 64)
        for p in range(3):
            _interleave_heads(tmpa, p * 224, wpt, p * 224)

    def prep_wo(anchor):
        u = padded_bits(woa_v[...])
        for r in range(DH):
            a = anchor(2 * r)
            for nt in range(4):
                tmpo[nt, 8 * r:8 * r + 8, :] = u[8 * r:8 * r + 8, nt * BL:(nt + 1) * BL] | a
        _interleave_heads(tmpo, 0, stack, 224)
        for j in range(4, 7):
            stack_t(j, anchor(60 + 30 * (j - 4)))

    def m_step(pace):
        zero = zeros_rt()
        tm = _bits(st['tm'])

        def anchor(i):
            return tm[8 * (i % 56):8 * (i % 56) + 8, (i // 56) * BL:(i // 56 + 1) * BL] & zero

        kk = _bits(jnp.concatenate(pk[12:NB], axis=0))
        prep_wo(lambda i: kk[8 * i:8 * i + 8] & zero)
        for j in range(4):
            transpose_cols(wb_v, 896 + j * BL, BL if j < 3 else 64, tmpv, j * 64)
        wv = _heads_f32(tmpv)
        u = padded_bits(wob_v[...])
        for r in range(DH):
            a = anchor(3 * r)
            for nt in range(4):
                tmpm[nt, 8 * r:8 * r + 8, :] = u[8 * r:8 * r + 8, nt * BL:(nt + 1) * BL] | a
        wo = _heads_f32(tmpm)
        for t in range(3):
            tt[t, 0:D, :] = st['tm'][:, t * BL:(t + 1) * BL]
        tt[3, 0:D, :] = jnp.concatenate([st['ts'], jnp.zeros((DP - D, D), F32)], axis=0).T
        pins = []
        for j in range(DH):
            for tab, i in ((wo, 100 + (j * 68) // DH), (wv, 30 + ((2 * j + 1) * 138) // (2 * DH))):
                b = _bits(tab[j])
                b = _tree(jnp.bitwise_or, [b[t, 8 * h:8 * h + 8] for t in range(4) for h in range(2)])
                pins.append(pltpu.roll(b & anchor(i), 1, 1))
        zero = zero | _tree(jnp.bitwise_or, pins)
        zero = jnp.concatenate([zero, zero], axis=0)
        p0, p1, first = 80, 1670, 56
        ngrp = (DH - 1) * (DH // JG)
        hist, mp, pinned = [], [], 0
        wvg = [jnp.stack(wv[j0:j0 + JG]) for j0 in range(0, DH, JG)]
        wog = [jnp.stack(wo[j0:j0 + JG]) for j0 in range(0, DH, JG)]
        for d in range(DH):
            td = _bits(tt[:, pl.ds(d, H, stride=DH), :])
            m = None
            for j0 in range(0, DH, JG):
                if d == 0:
                    pi = p0 + (j0 * first) // DH
                else:
                    pi = p0 + first + ((len(hist) - DH // JG) * (p1 - p0 - first)) // ngrp
                pv, pr_ = pace[pi // 2]
                zg = zero & _bits(pv[pr_])
                if pi >= 112 * pinned + 96:
                    zg = zg & _bits(rl_s[pinned])
                    pinned += 1
                tie = (_bits(hist[-2]) & zg[None]) if len(hist) >= 2 else zg[None]
                tg = pltpu.bitcast(td | tie, F32)
                pr = tg[None] * wvg[j0 // JG]
                kv = jnp.sum((pr[:, 0] + pr[:, 1]) + (pr[:, 2] + pr[:, 3]), axis=2, keepdims=True)
                p = kv[:, None] * wog[j0 // JG]
                if m is not None:
                    p = jnp.concatenate([m[None], p], axis=0)
                m = jnp.sum(p, axis=0)
                hist.append(m)
            mp.append(m)
        mp = [_bits(m.astype(BF16)) for m in mp]
        last = mp[-1][0] & zero[0:8]
        for d in range(DH):
            stack[:, 8 * d:8 * d + 8, :] = (mp[d] | last[None]) if d % 8 == 0 else mp[d]
        for j in range(4):
            stack_t(j)

    def proj(c, parts):
        x = xblk(c)
        if parts == (3, 0):
            rr = _dot(jnp.concatenate([_lanes(wpt, p * 224, 224, 4)[:, 0:D] for p in parts], axis=0), x)
        for ip, p in enumerate(parts):
            r = rr[ip * D:(ip + 1) * D] if parts == (3, 0) else _dot(_lanes(wpt, p * 224, 224, 4)[:, 0:D], x)
            if p == 0:
                q_s[c] = r.reshape(DH, H, BL)
            elif p == 1:
                k_s[c] = r.reshape(DH, H, BL)
                kp_s[c] = _bits(r.astype(BF16)).reshape(DH, 8, BL)
            elif p == 2:
                vp_s[c] = _bits(r.astype(BF16)).reshape(DH, 8, BL)
            else:
                qb_s[c] = r.reshape(DH, H, BL)
                pq_s[c] = _phi(r).reshape(DH, H, BL)

    def masks(ln):
        return [None] + [jnp.broadcast_to((ln >= BL - DIL * w)[None], (DH, 8, BL)) for w in range(1, W)]

    def shifted(vals, c, w, msk):
        cur = vals[c]
        if w > 0:
            if c > 0:
                cur = lax.select(msk[w], vals[c - 1], cur)
            cur = pltpu.roll(cur, DIL * w, 2)
        return pltpu.bitcast(cur, BF16).astype(F32)

    def attn(c):
        logit = []
        for w in range(W):
            k = k_s[c] if w == 0 else shifted(kp_s, c, w, st['msk'])
            logit.append(jnp.sum(q_s[c] * k, axis=0))
        if c == 0:
            logit = [jnp.where(lane16 >= DIL * w, l, -1e9 * DH ** 0.5) for w, l in enumerate(logit)]
        m = _tree(jnp.maximum, logit)
        e = [jnp.exp2((l - m) * (DH ** -0.5 * LOG2E)) for l in logit]
        r = g_s[c] / _tree(jnp.add, e)
        mb = pltpu.bitcast(m, jnp.int32)
        msk = masks(lane | (mb[0:8] & mb[8:16] & pltpu.bitcast(zeros_rt(), jnp.int32)))
        o = None
        for w in range(W):
            p = e[w][None] * shifted(vp_s, c, w, msk)
            o = p if o is None else o + p
        ua_s[c] = o * r[None]

    def lin(c):
        pq = pq_s[c]
        den = jnp.sum(pq * st['zb'], axis=0) + 1e-6
        rl_s[c] = (1.0 - g_s[c]) / den
        ub_s[c] = pq * rl_s[c][None]

    cp_o = []

    def final(c):
        u = jnp.concatenate([ub_s[c], ua_s[c]], axis=0).reshape(2 * D, BL)
        u0, u1 = u[0:384].astype(BF16), u[384:].astype(BF16)
        wl = [_lanes(wcat, 56 * i, 56, 7) for i in range(4)]
        o = []
        for i0 in (0, 2):
            pb = [_dot(wl[i][:, 0:384], u0) for i in (i0, i0 + 1)]
            if c == NB - 1:
                o += [_dot(wl[i][:, 384:], u1) + pb[i - i0] for i in (i0, i0 + 1)]
            else:
                o.append(_dot(_lanes(wcat, 56 * i0, 112, 7)[:, 384:], u1) + jnp.concatenate(pb, axis=0))
        o = jnp.concatenate(o, axis=0)
        cuts = (0, 112, 224, 336, 400, 432, D) if c == NB - 1 else (0, D)
        for r0, r1 in zip(cuts[:-1], cuts[1:]):
            o_s[c, r0:r1, :] = o[r0:r1].astype(BF16)
            cp = cpy(o_s.at[c, r0:r1, :], out_hbm.at[r0:r1, c * BL:(c + 1) * BL], sem.at[0])
            cp.start()
            cp_o.append(cp)

    wait(g0)
    for j in (2, 3):
        transpose_cols(wb_v, 384 + j * BL, BL, wkt, j * 64)
    wait(g1)
    whi = _lanes(wkt, 128, 128, 4)[:, 0:D]
    khi = [_phi(_dot(whi, xblk(c))) for c in range(2)]
    thi = [None, None]
    for c in range(2):
        for i in range(2):
            t = _dot_nt(khi[c][i * BL:(i + 1) * BL].astype(BF16), xs[0:384, c * BL:(c + 1) * BL])
            thi[i] = t if thi[i] is None else t + thi[i]
    wait(g2)
    khi += [_phi(_dot(whi, xblk(c))) for c in range(2, 4)]
    for j in (0, 1):
        transpose_cols(wb_v, 384 + j * BL, BL, wkt, j * 64)
    wlo = _lanes(wkt, 32, 96, 4)[:, 0:D]
    klo = [_phi(_dot(wlo, xblk(c))) for c in range(4)]
    for c in range(4):
        pk[c] = jnp.concatenate([klo[c], khi[c]], axis=0)
    for i in range(2):
        a = jnp.concatenate([khi[2][i * BL:(i + 1) * BL], khi[3][i * BL:(i + 1) * BL]], axis=1)
        thi[i] = _dot_nt(a.astype(BF16), xs[0:384, 2 * BL:4 * BL]) + thi[i]
    tlo = _dot_nt(jnp.concatenate(klo, axis=1).astype(BF16), xs[0:384, 0:4 * BL])
    st['tm'] = jnp.concatenate([tlo] + thi, axis=0)
    st['ts'] = _dot_nt(xs[384:D, 0:4 * BL], jnp.concatenate(pk[0:4], axis=1).astype(BF16))
    st['z'] = _tree(jnp.add, pk[0:4])
    st['gw'] = jnp.broadcast_to(g_v[...].astype(F32).reshape(1, D), (BL, D)).T
    wait(g3)
    for c in range(4, 9):
        kproj(c)
    tdot(4, 8)
    for c in range(9, 12):
        kproj(c)
    tdot(8, 12)
    wait(g4)
    prep()
    for c in range(12, NB):
        kproj(c)
    tdot(12, NB)
    z_step()
    pace = []
    for c in range(NW):
        proj(c, (3, 0))
        lin(c)
        pace += [(qb_s[c], i) for i in range(DH)] + [(q_s[c], i) for i in range(DH)]
    m_step(pace)
    st['msk'] = masks(lane)
    rest = [(c, p) for c in range(NW, NB) for p in (3, 0)]
    proj(0, (1,))
    proj(rest[0][0], (rest[0][1],))
    proj(0, (2,))
    attn(0)
    for c, p in rest[1:]:
        proj(c, (p,))
    for c in range(NW, NB):
        lin(c)
    for c in range(1, NB):
        proj(c, (2, 1) if c < NB - 1 else (1, 2))
        attn(c)
        final(c - 1)
    final(NB - 1)
    assert len(cp_o) == NB + 5
    wait(cp_o)


@jax.jit
def pallas_gated_mix__sliding_local_dilated__linear_attn_block__prompt_kernel(
        A_x, A_wqkv, A_wo, B_x, B_wqkv, B_wo, gate_w):
    del B_x
    xt = jnp.swapaxes(A_x, 1, 2).reshape(D, S)
    any_spec = pl.BlockSpec(memory_space=pl.ANY)
    V = pltpu.VMEM
    ot = pl.pallas_call(
        _kernel,
        out_shape=jax.ShapeDtypeStruct((D, S), BF16),
        grid=(2,),
        in_specs=[any_spec] * 6,
        out_specs=any_spec,
        scratch_shapes=[
            V((D, S + BL), BF16),
            V((DP, 3 * D), BF16),
            V((DP, 3 * D), BF16),
            V((D, D), BF16),
            V((D, D), BF16),
            V((D,), BF16),
            V((4, 256, BL), U32),
            V((4, 704, BL), U32),
            V((4, 256, BL), U32),
            V((4, 896, BL), U32),
            V((4, 256, BL), U32),
            V((4, 240, BL), U32),
            V((4, 240, BL), U32),
            V((4, 480, BL), F32),
            V((4, 448, BL), U32),
            V((7, 224, BL), U32),
            V((480, BL), F32),
            V((NB, D, BL), BF16),
            pltpu.SemaphoreType.DMA((5,)),
        ],
        compiler_params=pltpu.CompilerParams(dimension_semantics=("arbitrary",),
                                             vmem_limit_bytes=64 * 1024 * 1024,
                                             disable_semaphore_checks=True),
    )(xt, A_wqkv, A_wo, B_wqkv, B_wo, gate_w)
    return jnp.swapaxes(ot.reshape(1, D, S), 1, 2)
```
